```python
import jax
import jax.numpy as jnp

def _softmax(x, axis=-1):
    return jax.nn.softmax(x, axis=axis)

def _gelu(x):
    return jax.nn.gelu(x, approximate=True)

def _silu(x):
    return jax.nn.silu(x)

def _sigmoid(x):
    return jax.nn.sigmoid(x)

def _layernorm(x, axis=-1, eps=1e-05):
    m = jnp.mean(x, axis=axis, keepdims=True)
    v = jnp.var(x, axis=axis, keepdims=True)
    return (x - m) / jnp.sqrt(v + eps)

def _scatter_add(tgt, idx, src, axis=0):
    return tgt.at[idx].add(src)

def _segment_sum(src, seg, n):
    return jax.ops.segment_sum(src, seg, n)

class _Rng:

    def __init__(self, key):
        self._k = key

    def _next(self):
        self._k, sub = jax.random.split(self._k)
        return sub

    def normal(self, shape):
        return jax.random.normal(self._next(), shape, dtype=jnp.bfloat16)

    def randint(self, lo, hi, shape):
        return jax.random.randint(self._next(), shape, lo, hi, dtype=jnp.int32)

    def uniform(self, shape, lo=0.0, hi=1.0):
        return jax.random.uniform(self._next(), shape, jnp.bfloat16, lo, hi)

    def permutation(self, n):
        return jax.random.permutation(self._next(), n)
kernel_name = 'gated_mix__softmax_full_mha__memory_aug_recurrent_mem_tr__prompt'

def setup_inputs():
    _rng = _Rng(jax.random.key(int.from_bytes(__import__("os").urandom(4), "little")))
    _w = lambda a: (lambda t: t.astype(jnp.bfloat16) if jnp.issubdtype(t.dtype, jnp.floating) else t)(jnp.asarray(a))

    def _A_setup():
        B, S, D = (1, 2048, 1024)
        return {'x': _w((lambda *s: _rng.normal(s) * 0.05)(B, S, D)), 'wqkv': _w((lambda *s: _rng.normal(s) * 0.05)(D, 3 * D)), 'wo': _w((lambda *s: _rng.normal(s) * 0.05)(D, D))}
    _A_in = _A_setup()

    def _B_setup():
        B, S, Dm = (1, 2048, 1024)
        H, Dh = (32, 128)
        M, seg = (8, 32)
        seg = min(seg, S)
        S = S // seg * seg
        return {'x': _w((lambda *s: _rng.normal(s) * 0.05)(B, S, Dm)), 'mem0': _w((lambda *s: _rng.normal(s) * 0.05)(B, M, Dm)), 'Wq': _w((lambda *s: _rng.normal(s) * 0.05)(Dm, H, Dh) * Dm ** (-0.5)), 'Wk': _w((lambda *s: _rng.normal(s) * 0.05)(Dm, H, Dh) * Dm ** (-0.5)), 'Wv': _w((lambda *s: _rng.normal(s) * 0.05)(Dm, H, Dh) * Dm ** (-0.5)), 'Wo': _w((lambda *s: _rng.normal(s) * 0.05)(H, Dh, Dm) * (H * Dh) ** (-0.5)), 'seg_len': seg}
    _B_in = _B_setup()
    return {'A_x': _A_in['x'], 'A_wqkv': _A_in['wqkv'], 'A_wo': _A_in['wo'], 'B_x': _B_in['x'], 'B_mem0': _B_in['mem0'], 'B_Wq': _B_in['Wq'], 'B_Wk': _B_in['Wk'], 'B_Wv': _B_in['Wv'], 'B_Wo': _B_in['Wo'], 'B_seg_len': _B_in['seg_len'], 'gate_w': _w((lambda *s: _rng.normal(s) * 0.05)(1024))}

def reference(A_x, A_wqkv, A_wo, B_x, B_mem0, B_Wq, B_Wk, B_Wv, B_Wo, B_seg_len, gate_w):

    def _A_ref(x, wqkv, wo):
        B, S, D = x.shape
        H = 32
        Dh = D // H
        qkv = (lambda x, *d: x.transpose(*d))((x @ wqkv).reshape(B, S, 3, H, Dh), 2, 0, 3, 1, 4)
        q, k, v = (qkv[0], qkv[1], qkv[2])
        scale = Dh ** (-0.5)
        scores = jnp.einsum('bhqd,bhkd->bhqk', q, k) * scale
        p = _softmax(scores, axis=-1)
        o = jnp.einsum('bhqk,bhkd->bhqd', p, v)
        return (lambda x, *d: x.transpose(*d))(o, 0, 2, 1, 3).reshape(B, S, D) @ wo

    def _B_ref(x, mem0, Wq, Wk, Wv, Wo, seg_len):
        B, S, Dm = x.shape
        H, Dh = (Wq.shape[1], Wq.shape[2])
        M = mem0.shape[1]
        scale = Dh ** (-0.5)
        n_seg = S // seg_len
        L = M + seg_len
        idx = jnp.arange(L)
        mask = (idx[:, None] < M) | (idx[:, None] >= idx[None, :])
        mem = mem0
        outs = []
        for s in range(n_seg):
            xs = x[:, s * seg_len:(s + 1) * seg_len, :].copy()
            h = jnp.concatenate([mem, xs], axis=1)
            q = jnp.einsum('btd,dhe->bhte', h, Wq)
            k = jnp.einsum('btd,dhe->bhte', h, Wk)
            v = jnp.einsum('btd,dhe->bhte', h, Wv)
            scores = jnp.einsum('bhqe,bhke->bhqk', q, k) * scale
            scores = jnp.where(mask[None, None], scores, -1000000000.0)
            p = _softmax(scores, axis=-1)
            o = jnp.einsum('bhqk,bhke->bhqe', p, v)
            o = jnp.einsum('bhte,hed->btd', o, Wo)
            mem = o[:, :M, :].copy()
            outs.append(o[:, M:, :])
        return jnp.concatenate(outs, axis=1)
    x = A_x
    g = _sigmoid((x * gate_w).sum(-1, keepdims=True))
    a = _A_ref(x, A_wqkv, A_wo)
    b = _B_ref(x, B_mem0, B_Wq, B_Wk, B_Wv, B_Wo, B_seg_len)
    return g * a + (1 - g) * b
```

```python
import functools
import math

import jax
import jax.numpy as jnp
import jax.experimental.pallas as pl
import jax.experimental.pallas.tpu as pltpu

BF = jnp.bfloat16
F32 = jnp.float32
U32 = jnp.uint32

S = 2048
D = 1024
HA, DHA = 32, 32
HB, DHB = 32, 128
M = 8
SEG = 32
L = M + SEG

LOG2E = math.log2(math.e)
CA = DHA ** -0.5 * LOG2E
CB = DHB ** -0.5 * LOG2E
NEG_B = -1e9 * LOG2E

TB = 512
QB = 512
KB = 128
AHEAD = 2
GB = 4
NGB = HB // GB


def _tree(op, xs):
    xs = list(xs)
    while len(xs) > 1:
        nxt = [op(xs[i], xs[i + 1]) for i in range(0, len(xs) - 1, 2)]
        if len(xs) % 2:
            nxt.append(xs[-1])
        xs = nxt
    return xs[0]


def _kernel(ax_hbm, wqkv_hbm, awo_hbm, bx_hbm, mem_ref, bwq_hbm, bwk_hbm, bwv_hbm,
            bwo_hbm, gw_ref, out_hbm,
            ax, wqkv, awo, bx, kbuf, qt, vt, ot, abuf, gbuf, wb, wob, stage, outbuf,
            sem_in, sem_st, sem_out):
    nblk = S // TB

    def ax_cp(i):
        r0 = pl.multiple_of(i * TB, TB)
        return pltpu.make_async_copy(ax_hbm.at[pl.ds(r0, TB), :], ax.at[pl.ds(r0, TB), :],
                                     sem_in.at[i])

    def wqkv_cp(t):
        return pltpu.make_async_copy(wqkv_hbm.at[:, pl.ds(t * D, D)], wqkv.at[t],
                                     sem_in.at[nblk + t])

    awo_cp = pltpu.make_async_copy(awo_hbm, awo, sem_in.at[nblk + 3])
    bx_cp = pltpu.make_async_copy(bx_hbm, bx, sem_in.at[nblk + 4])
    wob_cp = pltpu.make_async_copy(bwo_hbm.bitcast(U32), wob, sem_in.at[nblk + 5])

    bw_u32 = [r.bitcast(U32) for r in (bwq_hbm, bwk_hbm, bwv_hbm)]

    def stage_cp(piece, slot, t):
        hp = piece // 2
        d0 = pl.multiple_of((piece % 2) * (D // 2), D // 2)
        return pltpu.make_async_copy(bw_u32[t].at[pl.ds(d0, D // 2), hp, :],
                                     stage.at[slot, t], sem_st.at[slot, t])

    ax_cp(0).start()
    wqkv_cp(1).start()
    for i in range(1, nblk):
        ax_cp(i).start()
    wqkv_cp(0).start()
    wqkv_cp(2).start()
    awo_cp.start()
    for t in range(3):
        stage_cp(0, 0, t).start()
    bx_cp.start()
    wob_cp.start()

    wqkv_cp(1).wait()

    def k_proj(i, c):
        ax_cp(i).wait()
        r0 = pl.multiple_of(i * TB, TB)
        xb = ax[pl.ds(r0, TB), :]
        kbuf[pl.ds(r0, TB), :] = jnp.dot(xb, wqkv[1], preferred_element_type=F32).astype(BF)
        gb = jnp.broadcast_to(gw_ref[...], (128, D))
        z = jax.lax.dot_general(xb, gb, (((1,), (1,)), ((), ())), preferred_element_type=F32)
        gbuf[pl.ds(r0, TB), :] = 1.0 / (1.0 + jnp.exp(-z))
        return c

    jax.lax.fori_loop(0, nblk, k_proj, 0)

    wqkv_cp(0).wait()
    wqkv_cp(2).wait()

    def qv_proj(i, c):
        r0 = pl.multiple_of(i * TB, TB)
        xb = ax[pl.ds(r0, TB), :]
        q = jnp.dot(xb, wqkv[0], preferred_element_type=F32) * CA
        qt[:, pl.ds(r0, TB)] = q.T.astype(BF)
        v = jnp.dot(xb, wqkv[2], preferred_element_type=F32)
        vt[:, pl.ds(r0, TB)] = v.T.astype(BF)
        return c

    jax.lax.fori_loop(0, nblk, qv_proj, 0)

    nq = S // QB
    nk = S // KB
    n_it = (HA // 4) * nq

    def attn_iter(it, c):
        slot = it % 2

        @pl.when(it + 1 < n_it)
        def _():
            for t in range(3):
                stage_cp(it + 1, 1 - slot, t).start()

        for t in range(3):
            stage_cp(it, slot, t).wait()

        r0 = pl.multiple_of((it % 2) * (D // 4), D // 4)
        for t in range(3):
            ev = stage[slot, t, pl.ds(0, D // 4, stride=2), :]
            od = stage[slot, t, pl.ds(1, D // 4, stride=2), :]
            lo = (ev & U32(0xFFFF)) | (od << 16)
            hi = (ev >> 16) | (od & U32(0xFFFF0000))
            c0 = pl.multiple_of((it // 2) * 768 + t * 128, 128)
            wb[pl.ds(r0, D // 4), pl.ds(c0, 128)] = lo
            wb[pl.ds(r0, D // 4), pl.ds(c0 + 384, 128)] = hi

        g = it // nq
        q0 = pl.multiple_of((it % nq) * QB, QB)
        g0 = pl.multiple_of(g * 128, 128)
        qg = qt[pl.ds(g0, 128), pl.ds(q0, QB)]
        qms = []
        for hh in range(4):
            parts = []
            if hh > 0:
                parts.append(jnp.zeros((32 * hh, QB), BF))
            parts.append(qg[32 * hh:32 * hh + 32])
            if hh < 3:
                parts.append(jnp.zeros((96 - 32 * hh, QB), BF))
            qms.append(jnp.concatenate(parts, axis=0))

        items = [(hh, j) for hh in range(4) for j in range(nk)]
        n = len(items)

        def qk(i):
            hh, j = items[i]
            kb = kbuf[j * KB:(j + 1) * KB, pl.ds(g0, 128)]
            return jnp.dot(kb, qms[hh], preferred_element_type=F32)

        state = {}

        def pv(i, p, al, l):
            hh, j = items[i]
            h0 = pl.multiple_of(g0 + hh * 32, 32)
            d = jnp.dot(vt[pl.ds(h0, 32), j * KB:(j + 1) * KB], p, preferred_element_type=F32)
            acc = d if j == 0 else state["acc"] * al + d
            state["acc"] = acc
            if j == nk - 1:
                o = acc / jnp.sum(l, axis=0, keepdims=True)
                ot[pl.ds(h0, 32), pl.ds(q0, QB)] = o.astype(BF)

        ss = {i: qk(i) for i in range(AHEAD)}
        m = l = None
        pend = None
        for i, (hh, j) in enumerate(items):
            if i + AHEAD < n:
                ss[i + AHEAD] = qk(i + AHEAD)
            if pend is not None:
                pv(*pend)
            s = ss.pop(i)
            bm = _tree(jnp.maximum, [s[8 * r:8 * r + 8] for r in range(KB // 8)])
            bm = jnp.max(bm, axis=0, keepdims=True)
            if j == 0:
                m, al = bm, None
                p = jnp.exp2(s - m)
                l = _tree(jnp.add, [p[8 * r:8 * r + 8] for r in range(KB // 8)])
            else:
                mn = jnp.maximum(m, bm)
                al = jnp.exp2(m - mn)
                p = jnp.exp2(s - mn)
                l = l * al + _tree(jnp.add, [p[8 * r:8 * r + 8] for r in range(KB // 8)])
                m = mn
            pend = (i, p.astype(BF), al, l)
        pv(*pend)
        return c

    jax.lax.fori_loop(0, n_it, attn_iter, 0)

    awo_cp.wait()

    def a_out(i, c):
        r0 = pl.multiple_of(i * TB, TB)
        a = jax.lax.dot_general(ot[:, pl.ds(r0, TB)], awo[...], (((0,), (0,)), ((), ())),
                                preferred_element_type=F32)
        g = gbuf[pl.ds(r0, TB), :]
        abuf[pl.ds(r0, TB), :] = a * jnp.concatenate([g] * (D // 128), axis=1)
        return c

    jax.lax.fori_loop(0, nblk, a_out, 0)

    bx_cp.wait()
    wob_cp.wait()

    ri = jax.lax.broadcasted_iota(jnp.int32, (L, L), 0)
    ci = jax.lax.broadcasted_iota(jnp.int32, (L, L), 1)
    mask = (ri < M) | (ri >= ci)

    def qkv_dot(lhs, g):
        w = pltpu.bitcast(wb[:, g * GB * 384:(g + 1) * GB * 384], BF)
        return jnp.dot(lhs, w, preferred_element_type=F32)

    def qk_dots(rows):
        res = []
        for hh in range(GB):
            b = hh * 384
            q = (rows[:, b:b + 128] * CB).astype(BF)
            k = rows[:, b + 128:b + 256].astype(BF)
            v = rows[:, b + 256:b + 384].astype(BF)
            s = jax.lax.dot_general(q, k, (((1,), (1,)), ((), ())), preferred_element_type=F32)
            res.append((s, v))
        return res

    def pv_dots(sv):
        outs = []
        for s, v in sv:
            s = jnp.where(mask, s, NEG_B)
            mx = jnp.max(s, axis=1, keepdims=True)
            p = jnp.exp2(s - mx)
            l = jnp.sum(p, axis=1, keepdims=True)
            o = jnp.dot(p.astype(BF), v, preferred_element_type=F32)
            outs.append(o / l)
        return jnp.concatenate(outs, axis=1)

    def wo_dot(lhs, g):
        w = pltpu.bitcast(wob[g * GB * 64:(g + 1) * GB * 64, :], BF)
        return jnp.dot(lhs.astype(BF), w, preferred_element_type=F32)

    def run_step(lhs, rows_fn, wo_lhs_fn):
        qkv, sv, o = {}, {}, {}
        out = None
        qkv[0] = qkv_dot(lhs, 0)
        for g in range(NGB + 2):
            if g + 1 < NGB:
                qkv[g + 1] = qkv_dot(lhs, g + 1)
            if 0 <= g - 1 < NGB:
                o[g - 1] = pv_dots(sv[g - 1])
            if g < NGB:
                sv[g] = qk_dots(rows_fn(qkv[g], g))
            if 0 <= g - 2 < NGB:
                d = wo_dot(wo_lhs_fn(o[g - 2], g - 2), g - 2)
                out = d if out is None else out + d
        return out, qkv, o

    def pair(j, mem):
        t0 = pl.multiple_of(j * 2 * SEG, 2 * SEG)
        t1 = pl.multiple_of(j * 2 * SEG + SEG, SEG)
        x_e = bx[pl.ds(t0, 48), :].astype(F32)[:40]
        x_o = bx[pl.ds(t1, SEG), :].astype(F32)[8:]
        lhs_e = jnp.concatenate([mem, x_e], axis=0).astype(BF)
        out_e, qkv_e, o_e = run_step(lhs_e, lambda q, g: q[:L], lambda o, g: o[:32])
        mem1 = out_e[:M].astype(BF).astype(F32)
        lhs_o = jnp.concatenate([mem1, x_o], axis=0).astype(BF)
        out_o, _, _ = run_step(
            lhs_o,
            lambda q, g: jnp.concatenate([q[:8], qkv_e[g][40:48], q[8:32]], axis=0),
            lambda o, g: jnp.concatenate([o, o_e[g][32:40]], axis=0))
        b = jnp.concatenate([out_e[8:32], out_o[40:48], out_o[8:40]], axis=0)
        g = gbuf[pl.ds(t0, 2 * SEG), :]
        omg = jnp.concatenate([1.0 - g] * (D // 128), axis=1)
        outbuf[pl.ds(t0, 2 * SEG), :] = (abuf[pl.ds(t0, 2 * SEG), :] + omg * b).astype(BF)
        pltpu.make_async_copy(outbuf.at[pl.ds(t0, 2 * SEG), :],
                              out_hbm.at[pl.ds(t0, 2 * SEG), :], sem_out).start()
        return out_o[:M].astype(BF).astype(F32)

    jax.lax.fori_loop(0, S // (2 * SEG), pair, mem_ref[...].astype(F32))

    pltpu.make_async_copy(outbuf, out_hbm, sem_out).wait()


@functools.partial(jax.jit, static_argnames=("B_seg_len",))
def pallas_gated_mix__softmax_full_mha__memory_aug_recurrent_mem_tr__prompt_kernel(
    A_x: jax.Array,
    A_wqkv: jax.Array,
    A_wo: jax.Array,
    B_x: jax.Array,
    B_mem0: jax.Array,
    B_Wq: jax.Array,
    B_Wk: jax.Array,
    B_Wv: jax.Array,
    B_Wo: jax.Array,
    B_seg_len: int,
    gate_w: jax.Array,
):
    assert B_seg_len == SEG
    assert A_x.shape == (1, S, D) and B_x.shape == (1, S, D)
    assert B_Wq.shape == (D, HB, DHB) and B_Wo.shape == (HB, DHB, D)

    any_spec = pl.BlockSpec(memory_space=pl.ANY)
    vmem_spec = pl.BlockSpec(memory_space=pltpu.VMEM)
    out = pl.pallas_call(
        _kernel,
        out_shape=jax.ShapeDtypeStruct((S, D), BF),
        in_specs=[any_spec, any_spec, any_spec, any_spec, vmem_spec, any_spec, any_spec,
                  any_spec, any_spec, vmem_spec],
        out_specs=any_spec,
        scratch_shapes=[
            pltpu.VMEM((S, D), BF),
            pltpu.VMEM((3, D, D), BF),
            pltpu.VMEM((D, D), BF),
            pltpu.VMEM((S, D), BF),
            pltpu.VMEM((S, D), BF),
            pltpu.VMEM((D, S), BF),
            pltpu.VMEM((D, S), BF),
            pltpu.VMEM((D, S), BF),
            pltpu.VMEM((S, D), F32),
            pltpu.VMEM((S, 128), F32),
            pltpu.VMEM((D // 2, HB * 384), U32),
            pltpu.VMEM((HB * DHB // 2, D), U32),
            pltpu.VMEM((2, 3, D // 2, 128), U32),
            pltpu.VMEM((S, D), BF),
            pltpu.SemaphoreType.DMA((S // TB + 6,)),
            pltpu.SemaphoreType.DMA((2, 3)),
            pltpu.SemaphoreType.DMA(()),
        ],
        compiler_params=pltpu.CompilerParams(vmem_limit_bytes=120 * 1024 * 1024),
    )(A_x.reshape(S, D), A_wqkv, A_wo, B_x.reshape(S, D), B_mem0.reshape(M, D),
      B_Wq, B_Wk, B_Wv, B_Wo.reshape(HB * DHB, D), gate_w.reshape(1, D))
    return out.reshape(1, S, D)
```

```python
import functools
import math

import jax
import jax.numpy as jnp
import jax.experimental.pallas as pl
import jax.experimental.pallas.tpu as pltpu

BF = jnp.bfloat16
F32 = jnp.float32
U32 = jnp.uint32

S = 2048
D = 1024
HA, DHA = 32, 32
HB, DHB = 32, 128
M = 8
SEG = 32
L = M + SEG

LOG2E = math.log2(math.e)
CA = DHA ** -0.5 * LOG2E
CB = DHB ** -0.5 * LOG2E
NEG_B = -1e9 * LOG2E

TB = 512
QB = 256
KB = 128
AHEAD = 4
UN = 8
GB = 4
NGB = HB // GB
NQ = S // QB
NK = S // KB
N_UNITS = HA * NQ
N_PAIRS = S // (2 * SEG)
N_HP = HB // 2


def _tree(op, xs):
    xs = list(xs)
    while len(xs) > 1:
        nxt = [op(xs[i], xs[i + 1]) for i in range(0, len(xs) - 1, 2)]
        if len(xs) % 2:
            nxt.append(xs[-1])
        xs = nxt
    return xs[0]


def _kernel(ax_hbm, wqkv_hbm, awo_hbm, bx_hbm, mem_ref, bwq_hbm, bwk_hbm, bwv_hbm,
            bwo_hbm, gw_ref, out_hbm,
            ax, wqkv, awo, bx, kbuf, qt, vt, ot, abuf, gbuf, wb, wob, stage, outbuf, scarry,
            sem_in, sem_st, sem_out):
    nblk = S // TB

    def ax_cp(i):
        r0 = pl.multiple_of(i * TB, TB)
        return pltpu.make_async_copy(ax_hbm.at[pl.ds(r0, TB), :], ax.at[pl.ds(r0, TB), :],
                                     sem_in.at[i])

    def wqkv_cp(t):
        return pltpu.make_async_copy(wqkv_hbm.at[:, pl.ds(t * D, D)], wqkv.at[t],
                                     sem_in.at[nblk + t])

    awo_cp = pltpu.make_async_copy(awo_hbm, awo, sem_in.at[nblk + 3])
    bx_cp = pltpu.make_async_copy(bx_hbm, bx, sem_in.at[nblk + 4])
    wob_cp = pltpu.make_async_copy(bwo_hbm.bitcast(U32), wob, sem_in.at[nblk + 5])

    bw_u32 = [r.bitcast(U32) for r in (bwq_hbm, bwk_hbm, bwv_hbm)]

    def stage_cp(hp, t):
        return pltpu.make_async_copy(bw_u32[t].at[:, hp, :], stage.at[hp * 3 + t],
                                     sem_st.at[hp])

    ax_cp(0).start()
    wqkv_cp(1).start()
    wqkv_cp(1).wait()
    for i in range(1, nblk):
        ax_cp(i).start()
    wqkv_cp(0).start()
    wqkv_cp(2).start()

    def k_proj(i, c):
        ax_cp(i).wait()
        r0 = pl.multiple_of(i * TB, TB)
        xb = ax[pl.ds(r0, TB), :]
        kbuf[pl.ds(r0, TB), :] = jnp.dot(xb, wqkv[1], preferred_element_type=F32).astype(BF)
        z = jnp.sum(xb.astype(F32) * gw_ref[...].astype(F32), axis=1, keepdims=True)
        gbuf[pl.ds(r0, TB), :] = jnp.broadcast_to(1.0 / (1.0 + jnp.exp(-z)), (TB, 128))
        return c

    with jax.named_scope("ph_kproj"):
        jax.lax.fori_loop(0, nblk, k_proj, 0)

    for hp in range(N_HP):
        for t in range(3):
            stage_cp(hp, t).start()
    awo_cp.start()
    bx_cp.start()
    wob_cp.start()
    wqkv_cp(0).wait()
    wqkv_cp(2).wait()

    def qv_proj(i, c):
        r0 = pl.multiple_of(i * TB, TB)
        xb = ax[pl.ds(r0, TB), :]
        q = jnp.dot(xb, wqkv[0], preferred_element_type=F32) * CA
        qt[:, pl.ds(r0, TB)] = q.T.astype(BF)
        v = jnp.dot(xb, wqkv[2], preferred_element_type=F32)
        vt[:, pl.ds(r0, TB)] = v.T.astype(BF)
        return c

    with jax.named_scope("ph_qvproj"):
        jax.lax.fori_loop(0, nblk, qv_proj, 0)

    def unit_setup(u):
        h = u % HA
        g0 = pl.multiple_of((h // 4) * 128, 128)
        h0 = pl.multiple_of(h * DHA, DHA)
        q0 = pl.multiple_of((u // HA) * QB, QB)
        qg = pltpu.bitcast(qt[pl.ds(g0, 128), pl.ds(q0, QB)], U32)
        rows = jax.lax.broadcasted_iota(jnp.int32, (64, QB), 0)
        qm = pltpu.bitcast(jnp.where(rows // 16 == h % 4, qg, U32(0)), BF)
        return qm, g0, h0, q0

    def qk_chunk(setup, j):
        qm, g0, _, _ = setup
        kb = kbuf[j * KB:(j + 1) * KB, pl.ds(g0, 128)]
        return jnp.dot(kb, qm, preferred_element_type=F32)

    def attn_iter(it, c):
        setup = [unit_setup(it * UN + k) for k in range(UN)]
        setup_next = unit_setup(jnp.minimum(it * UN + UN, N_UNITS - 1))
        items = [(uu, j) for uu in range(UN) for j in range(NK)]
        n = len(items)
        state = {}

        def pv(i, p, al, l):
            uu, j = items[i]
            _, _, h0, q0 = setup[uu]
            d = jnp.dot(vt[pl.ds(h0, DHA), j * KB:(j + 1) * KB], p, preferred_element_type=F32)
            acc = d if j == 0 else state["acc"] * al + d
            state["acc"] = acc
            if j == NK - 1:
                o = acc / jnp.sum(l, axis=0, keepdims=True)
                ot[pl.ds(h0, DHA), pl.ds(q0, QB)] = o.astype(BF)

        ss = {i: scarry[i] for i in range(AHEAD)}
        m = l = None
        pend = None
        for i, (uu, j) in enumerate(items):
            if i + AHEAD < n:
                uu2, j2 = items[i + AHEAD]
                ss[i + AHEAD] = qk_chunk(setup[uu2], j2)
            else:
                scarry[i + AHEAD - n] = qk_chunk(setup_next, i + AHEAD - n)
            if pend is not None:
                pv(*pend)
            s = ss.pop(i)
            bm = _tree(jnp.maximum, [s[8 * r:8 * r + 8] for r in range(KB // 8)])
            bm = jnp.max(bm, axis=0, keepdims=True)
            if j == 0:
                m, al = bm, None
                p = jnp.exp2(s - m)
                l = _tree(jnp.add, [p[8 * r:8 * r + 8] for r in range(KB // 8)])
            else:
                mn = jnp.maximum(m, bm)
                al = jnp.exp2(m - mn)
                p = jnp.exp2(s - mn)
                l = l * al + _tree(jnp.add, [p[8 * r:8 * r + 8] for r in range(KB // 8)])
                m = mn
            pend = (i, p.astype(BF), al, l)
        pv(*pend)
        return c

    setup0 = unit_setup(0)
    for j in range(AHEAD):
        scarry[j] = qk_chunk(setup0, j)
    with jax.named_scope("ph_attn"):
        jax.lax.fori_loop(0, N_UNITS // UN, attn_iter, 0)

    awo_cp.wait()

    def a_out(i, c):
        r0 = pl.multiple_of(i * TB, TB)
        a = jax.lax.dot_general(ot[:, pl.ds(r0, TB)], awo[...], (((0,), (0,)), ((), ())),
                                preferred_element_type=F32)
        g = gbuf[pl.ds(r0, TB), :]
        abuf[pl.ds(r0, TB), :] = a * jnp.concatenate([g] * (D // 128), axis=1)
        return c

    with jax.named_scope("ph_aout"):
        jax.lax.fori_loop(0, nblk, a_out, 0)

    def relayout(hp, c):
        pltpu.make_async_copy(stage.at[pl.ds(hp * 3, 3)], stage.at[pl.ds(hp * 3, 3)],
                              sem_st.at[hp]).wait()
        for t in range(3):
            ev = stage[hp * 3 + t, pl.ds(0, D // 2, stride=2), :]
            od = stage[hp * 3 + t, pl.ds(1, D // 2, stride=2), :]
            lo = (ev & U32(0xFFFF)) | (od << 16)
            hi = (ev >> 16) | (od & U32(0xFFFF0000))
            c0 = pl.multiple_of(hp * 768 + t * 128, 128)
            wb[:, pl.ds(c0, 128)] = lo
            wb[:, pl.ds(c0 + 384, 128)] = hi
        return c

    with jax.named_scope("ph_relayout"):
        jax.lax.fori_loop(0, N_HP, relayout, 0)

    bx_cp.wait()
    wob_cp.wait()

    ri = jax.lax.broadcasted_iota(jnp.int32, (L, L), 0)
    ci = jax.lax.broadcasted_iota(jnp.int32, (L, L), 1)
    mask = (ri < M) | (ri >= ci)

    def qkv_dot(lhs, g):
        w = pltpu.bitcast(wb[:, g * GB * 384:(g + 1) * GB * 384], BF)
        return jnp.dot(lhs, w, preferred_element_type=F32)

    def qk_dots(rows):
        res = []
        for hh in range(GB):
            b = hh * 384
            q = (rows[:, b:b + 128] * CB).astype(BF)
            k = rows[:, b + 128:b + 256].astype(BF)
            v = rows[:, b + 256:b + 384].astype(BF)
            s = jax.lax.dot_general(q, k, (((1,), (1,)), ((), ())), preferred_element_type=F32)
            res.append((s, v))
        return res

    def pv_dots(sv):
        outs = []
        for s, v in sv:
            s = jnp.where(mask, s, NEG_B)
            mx = jnp.max(s, axis=1, keepdims=True)
            p = jnp.exp2(s - mx)
            l = jnp.sum(p, axis=1, keepdims=True)
            o = jnp.dot(p.astype(BF), v, preferred_element_type=F32)
            outs.append(o / l)
        return jnp.concatenate(outs, axis=1)

    def wo_dot(lhs, g):
        w = pltpu.bitcast(wob[g * GB * 64:(g + 1) * GB * 64, :], BF)
        return jnp.dot(lhs.astype(BF), w, preferred_element_type=F32)

    def run_step(lhs, rows_fn, wo_lhs_fn):
        qkv, sv, o = {}, {}, {}
        out = None
        qkv[0] = qkv_dot(lhs, 0)
        for g in range(NGB + 2):
            if g + 1 < NGB:
                qkv[g + 1] = qkv_dot(lhs, g + 1)
            if 0 <= g - 1 < NGB:
                o[g - 1] = pv_dots(sv[g - 1])
            if g < NGB:
                sv[g] = qk_dots(rows_fn(qkv[g], g))
            if 0 <= g - 2 < NGB:
                d = wo_dot(wo_lhs_fn(o[g - 2], g - 2), g - 2)
                out = d if out is None else out + d
        return out, qkv, o

    def pair(j, mem):
        t0 = pl.multiple_of(j * 2 * SEG, 2 * SEG)
        t1 = pl.multiple_of(j * 2 * SEG + SEG, SEG)
        x_e = bx[pl.ds(t0, 48), :].astype(F32)[:40]
        x_o = bx[pl.ds(t1, SEG), :].astype(F32)[8:]
        lhs_e = jnp.concatenate([mem, x_e], axis=0).astype(BF)
        out_e, qkv_e, o_e = run_step(
            lhs_e, lambda q, g: q[:L], lambda o, g: o[:32])
        mem1 = out_e[:M].astype(BF).astype(F32)
        lhs_o = jnp.concatenate([mem1, x_o], axis=0).astype(BF)
        out_o, _, _ = run_step(
            lhs_o,
            lambda q, g: jnp.concatenate([q[:8], qkv_e[g][40:48], q[8:32]], axis=0),
            lambda o, g: jnp.concatenate([o, o_e[g][32:40]], axis=0))
        b = jnp.concatenate([out_e[8:32], out_o[40:48], out_o[8:40]], axis=0)
        g = gbuf[pl.ds(t0, 2 * SEG), :]
        omg = jnp.concatenate([1.0 - g] * (D // 128), axis=1)
        outbuf[pl.ds(t0, 2 * SEG), :] = (abuf[pl.ds(t0, 2 * SEG), :] + omg * b).astype(BF)
        pltpu.make_async_copy(outbuf.at[pl.ds(t0, 2 * SEG), :],
                              out_hbm.at[pl.ds(t0, 2 * SEG), :], sem_out).start()
        return out_o[:M].astype(BF).astype(F32)

    with jax.named_scope("ph_pair"):
        jax.lax.fori_loop(0, N_PAIRS, pair, mem_ref[...].astype(F32))

    pltpu.make_async_copy(outbuf, out_hbm, sem_out).wait()


@functools.partial(jax.jit, static_argnames=("B_seg_len",))
def pallas_gated_mix__softmax_full_mha__memory_aug_recurrent_mem_tr__prompt_kernel(
    A_x: jax.Array,
    A_wqkv: jax.Array,
    A_wo: jax.Array,
    B_x: jax.Array,
    B_mem0: jax.Array,
    B_Wq: jax.Array,
    B_Wk: jax.Array,
    B_Wv: jax.Array,
    B_Wo: jax.Array,
    B_seg_len: int,
    gate_w: jax.Array,
):
    assert B_seg_len == SEG
    assert A_x.shape == (1, S, D) and B_x.shape == (1, S, D)
    assert B_Wq.shape == (D, HB, DHB) and B_Wo.shape == (HB, DHB, D)

    any_spec = pl.BlockSpec(memory_space=pl.ANY)
    vmem_spec = pl.BlockSpec(memory_space=pltpu.VMEM)
    out = pl.pallas_call(
        _kernel,
        out_shape=jax.ShapeDtypeStruct((S, D), BF),
        in_specs=[any_spec, any_spec, any_spec, any_spec, vmem_spec, any_spec, any_spec,
                  any_spec, any_spec, vmem_spec],
        out_specs=any_spec,
        scratch_shapes=[
            pltpu.VMEM((S, D), BF),
            pltpu.VMEM((3, D, D), BF),
            pltpu.VMEM((D, D), BF),
            pltpu.VMEM((S, D), BF),
            pltpu.VMEM((S, D), BF),
            pltpu.VMEM((D, S), BF),
            pltpu.VMEM((D, S), BF),
            pltpu.VMEM((D, S), BF),
            pltpu.VMEM((S, D), F32),
            pltpu.VMEM((S, 128), F32),
            pltpu.VMEM((D // 2, HB * 384), U32),
            pltpu.VMEM((HB * DHB // 2, D), U32),
            pltpu.VMEM((N_HP * 3, D, 128), U32),
            pltpu.VMEM((S, D), BF),
            pltpu.VMEM((AHEAD, KB, QB), F32),
            pltpu.SemaphoreType.DMA((S // TB + 6,)),
            pltpu.SemaphoreType.DMA((N_HP,)),
            pltpu.SemaphoreType.DMA(()),
        ],
        compiler_params=pltpu.CompilerParams(vmem_limit_bytes=124 * 1024 * 1024),
    )(A_x.reshape(S, D), A_wqkv, A_wo, B_x.reshape(S, D), B_mem0.reshape(M, D),
      B_Wq, B_Wk, B_Wv, B_Wo.reshape(HB * DHB, D), gate_w.reshape(1, D))
    return out.reshape(1, S, D)
```

```python
import functools
import math

import jax
import jax.numpy as jnp
import jax.experimental.pallas as pl
import jax.experimental.pallas.tpu as pltpu

BF = jnp.bfloat16
F32 = jnp.float32
U32 = jnp.uint32

S = 2048
D = 1024
HA, DHA = 32, 32
HB, DHB = 32, 128
M = 8
SEG = 32
L = M + SEG

LOG2E = math.log2(math.e)
CA = DHA ** -0.5 * LOG2E
CB = DHB ** -0.5 * LOG2E
NEG_B = -1e9 * LOG2E

TB = 512
QB = 256
KB = 128
AHEAD = 4
UN = 8
GB = 4
NGB = HB // GB
NQ = S // QB
NK = S // KB
N_UNITS = HA * NQ
N_PAIRS = S // (2 * SEG)
N_HP = HB // 2


def _tree(op, xs):
    xs = list(xs)
    while len(xs) > 1:
        nxt = [op(xs[i], xs[i + 1]) for i in range(0, len(xs) - 1, 2)]
        if len(xs) % 2:
            nxt.append(xs[-1])
        xs = nxt
    return xs[0]


def _kernel(ax_hbm, wqkv_hbm, awo_hbm, mem_ref, bwq_hbm, bwk_hbm, bwv_hbm,
            bwo_hbm, gw_ref, out_hbm,
            ax, wqkv, awo, kbuf, qt, vt, ot, abuf, gbuf, wb, wob, stage, outbuf, scarry,
            sem_in, sem_st, sem_out):
    nblk = S // TB

    def ax_cp(i):
        r0 = pl.multiple_of(i * TB, TB)
        return pltpu.make_async_copy(ax_hbm.at[pl.ds(r0, TB), :], ax.at[pl.ds(r0, TB), :],
                                     sem_in.at[i])

    def wqkv_cp(t):
        return pltpu.make_async_copy(wqkv_hbm.at[:, pl.ds(t * D, D)], wqkv.at[t],
                                     sem_in.at[nblk + t])

    awo_cp = pltpu.make_async_copy(awo_hbm, awo, sem_in.at[nblk + 3])
    wob_cp = pltpu.make_async_copy(bwo_hbm.bitcast(U32), wob, sem_in.at[nblk + 4])

    bw_u32 = [r.bitcast(U32) for r in (bwq_hbm, bwk_hbm, bwv_hbm)]

    def stage_cp(hp, t):
        return pltpu.make_async_copy(bw_u32[t].at[:, hp, :], stage.at[hp * 3 + t],
                                     sem_st.at[hp])

    ax_cp(0).start()
    wqkv_cp(1).start()
    wqkv_cp(1).wait()
    for i in range(1, nblk):
        ax_cp(i).start()
    wqkv_cp(0).start()
    wqkv_cp(2).start()

    def k_proj(i, c):
        ax_cp(i).wait()
        r0 = pl.multiple_of(i * TB, TB)
        xb = ax[pl.ds(r0, TB), :]
        kbuf[pl.ds(r0, TB), :] = jnp.dot(xb, wqkv[1], preferred_element_type=F32).astype(BF)
        z = jnp.sum(xb.astype(F32) * gw_ref[...].astype(F32), axis=1, keepdims=True)
        gbuf[pl.ds(r0, TB), :] = jnp.broadcast_to(1.0 / (1.0 + jnp.exp(-z)), (TB, 128))
        return c

    with jax.named_scope("ph_kproj"):
        jax.lax.fori_loop(0, nblk, k_proj, 0)

    def start_rest():
        for hp in range(N_HP):
            for t in range(3):
                stage_cp(hp, t).start()
        awo_cp.start()
        wob_cp.start()
    start_rest()
    wqkv_cp(0).wait()
    wqkv_cp(2).wait()

    def qv_proj(i, c):
        r0 = pl.multiple_of(i * TB, TB)
        xb = ax[pl.ds(r0, TB), :]
        q = jnp.dot(xb, wqkv[0], preferred_element_type=F32) * CA
        qt[:, pl.ds(r0, TB)] = q.T.astype(BF)
        v = jnp.dot(xb, wqkv[2], preferred_element_type=F32)
        vt[:, pl.ds(r0, TB)] = v.T.astype(BF)
        return c

    with jax.named_scope("ph_qvproj"):
        jax.lax.fori_loop(0, nblk, qv_proj, 0)

    def unit_setup(u):
        h = u % HA
        g0 = pl.multiple_of((h // 4) * 128, 128)
        h0 = pl.multiple_of(h * DHA, DHA)
        q0 = pl.multiple_of((u // HA) * QB, QB)
        qg = pltpu.bitcast(qt[pl.ds(g0, 128), pl.ds(q0, QB)], U32)
        rows = jax.lax.broadcasted_iota(jnp.int32, (64, QB), 0)
        qm = pltpu.bitcast(jnp.where(rows // 16 == h % 4, qg, U32(0)), BF)
        return qm, g0, h0, q0

    def qk_chunk(setup, j):
        qm, g0, _, _ = setup
        kb = kbuf[j * KB:(j + 1) * KB, pl.ds(g0, 128)]
        return jnp.dot(kb, qm, preferred_element_type=F32)

    def attn_iter(it, c):
        setup = [unit_setup(it * UN + k) for k in range(UN)]
        setup_next = unit_setup(jnp.minimum(it * UN + UN, N_UNITS - 1))
        items = [(uu, j) for uu in range(UN) for j in range(NK)]
        n = len(items)
        state = {}

        def pv(i, p, al, l):
            uu, j = items[i]
            _, _, h0, q0 = setup[uu]
            d = jnp.dot(vt[pl.ds(h0, DHA), j * KB:(j + 1) * KB], p, preferred_element_type=F32)
            acc = d if j == 0 else state["acc"] * al + d
            state["acc"] = acc
            if j == NK - 1:
                o = acc / jnp.sum(l, axis=0, keepdims=True)
                ot[pl.ds(h0, DHA), pl.ds(q0, QB)] = o.astype(BF)

        ss = {i: scarry[i] for i in range(AHEAD)}
        m = l = None
        pend = None
        for i, (uu, j) in enumerate(items):
            if i + AHEAD < n:
                uu2, j2 = items[i + AHEAD]
                ss[i + AHEAD] = qk_chunk(setup[uu2], j2)
            else:
                scarry[i + AHEAD - n] = qk_chunk(setup_next, i + AHEAD - n)
            if pend is not None:
                pv(*pend)
            s = ss.pop(i)
            bm = _tree(jnp.maximum, [s[8 * r:8 * r + 8] for r in range(KB // 8)])
            bm = jnp.max(bm, axis=0, keepdims=True)
            if j == 0:
                m, al = bm, None
                p = jnp.exp2(s - m)
                l = _tree(jnp.add, [p[8 * r:8 * r + 8] for r in range(KB // 8)])
            else:
                mn = jnp.maximum(m, bm)
                al = jnp.exp2(m - mn)
                p = jnp.exp2(s - mn)
                l = l * al + _tree(jnp.add, [p[8 * r:8 * r + 8] for r in range(KB // 8)])
                m = mn
            pend = (i, p.astype(BF), al, l)
        pv(*pend)
        return c

    setup0 = unit_setup(0)
    for j in range(AHEAD):
        scarry[j] = qk_chunk(setup0, j)
    with jax.named_scope("ph_attn"):
        jax.lax.fori_loop(0, N_UNITS // UN, attn_iter, 0)

    awo_cp.wait()

    def a_out(i, c):
        r0 = pl.multiple_of(i * TB, TB)
        a = jax.lax.dot_general(ot[:, pl.ds(r0, TB)], awo[...], (((0,), (0,)), ((), ())),
                                preferred_element_type=F32)
        g = gbuf[pl.ds(r0, TB), :]
        abuf[pl.ds(r0, TB), :] = a * jnp.concatenate([g] * (D // 128), axis=1)
        return c

    with jax.named_scope("ph_aout"):
        jax.lax.fori_loop(0, nblk, a_out, 0)

    def relayout(hp, c):
        pltpu.make_async_copy(stage.at[pl.ds(hp * 3, 3)], stage.at[pl.ds(hp * 3, 3)],
                              sem_st.at[hp]).wait()
        for t in range(3):
            ev = stage[hp * 3 + t, pl.ds(0, D // 2, stride=2), :]
            od = stage[hp * 3 + t, pl.ds(1, D // 2, stride=2), :]
            lo = (ev & U32(0xFFFF)) | (od << 16)
            hi = (ev >> 16) | (od & U32(0xFFFF0000))
            c0 = pl.multiple_of(hp * 768 + t * 128, 128)
            wb[:, pl.ds(c0, 128)] = lo
            wb[:, pl.ds(c0 + 384, 128)] = hi
        return c

    with jax.named_scope("ph_relayout"):
        jax.lax.fori_loop(0, N_HP, relayout, 0)

    wob_cp.wait()

    NE, NO = 32, 48
    ri = jax.lax.broadcasted_iota(jnp.int32, (NE, L), 0)
    ci = jax.lax.broadcasted_iota(jnp.int32, (NE, L), 1)
    mask_e = (ri < M) | (ri >= ci)
    fill_e = NEG_B
    ri = jax.lax.broadcasted_iota(jnp.int32, (NO, 2 * L), 0)
    ci = jax.lax.broadcasted_iota(jnp.int32, (NO, 2 * L), 1)
    own = ((ri < L) & (ci >= L)) | ((ri >= L) & (ci < L))
    qi = jnp.where(ri < L, ri, ri - 8)
    ki = jnp.where(ci < L, ci, ci - L)
    mask_o = own & ((qi < M) | (qi >= ki))
    fill_o = jnp.where(own, NEG_B, -3e38)

    def qkv_dot(lhs, g):
        w = pltpu.bitcast(wb[:, g * GB * 384:(g + 1) * GB * 384], BF)
        return jnp.dot(lhs, w, preferred_element_type=F32)

    def qk_dots(qrows, kvrows):
        res = []
        for hh in range(GB):
            b = hh * 384
            q = (qrows[:, b:b + 128] * CB).astype(BF)
            k = kvrows[:, b + 128:b + 256].astype(BF)
            v = kvrows[:, b + 256:b + 384].astype(BF)
            s = jax.lax.dot_general(q, k, (((1,), (1,)), ((), ())), preferred_element_type=F32)
            res.append((s, v))
        return res

    def pv_dots(sv, mask, fill):
        outs = []
        for s, v in sv:
            s = jnp.where(mask, s, fill)
            mx = jnp.max(s, axis=1, keepdims=True)
            p = jnp.exp2(s - mx)
            l = jnp.sum(p, axis=1, keepdims=True)
            o = jnp.dot(p.astype(BF), v, preferred_element_type=F32)
            outs.append(o / l)
        return jnp.concatenate(outs, axis=1)

    def wo_dot(lhs, g):
        w = pltpu.bitcast(wob[g * GB * 64:(g + 1) * GB * 64, :], BF)
        return jnp.dot(lhs.astype(BF), w, preferred_element_type=F32)

    def run_step(lhs, rows_fn, mask, fill):
        qkv, sv, o = {}, {}, {}
        out = None
        qkv[0] = qkv_dot(lhs, 0)
        for g in range(NGB + 2):
            if g + 1 < NGB:
                qkv[g + 1] = qkv_dot(lhs, g + 1)
            if 0 <= g - 1 < NGB:
                o[g - 1] = pv_dots(sv[g - 1], mask, fill)
            if g < NGB:
                sv[g] = qk_dots(*rows_fn(qkv[g], g))
            if 0 <= g - 2 < NGB:
                d = wo_dot(o[g - 2], g - 2)
                out = d if out is None else out + d
        return out, qkv

    def pair(j, mem):
        t0 = pl.multiple_of(j * 2 * SEG, 2 * SEG)
        t1 = pl.multiple_of(j * 2 * SEG + SEG, SEG)
        x_e = ax[pl.ds(t0, 48), :].astype(F32)[:40]
        x_o = ax[pl.ds(t1, SEG), :].astype(F32)[8:]
        lhs_e = jnp.concatenate([mem, x_e], axis=0).astype(BF)
        out_e, qkv_e = run_step(lhs_e, lambda q, g: (q[:NE], q[:L]), mask_e, fill_e)
        mem1 = out_e[:M].astype(BF).astype(F32)
        lhs_o = jnp.concatenate([mem1, x_o], axis=0).astype(BF)

        def rows_o(q, g):
            e = qkv_e[g]
            seg_o = [q[:8], e[40:48], q[8:32]]
            return (jnp.concatenate(seg_o + [e[32:40]], axis=0),
                    jnp.concatenate([e[:L]] + seg_o, axis=0))

        out_o, _ = run_step(lhs_o, rows_o, mask_o, fill_o)
        b = jnp.concatenate([out_e[8:32], out_o[40:48], out_o[8:40]], axis=0)
        g = gbuf[pl.ds(t0, 2 * SEG), :]
        omg = jnp.concatenate([1.0 - g] * (D // 128), axis=1)
        outbuf[pl.ds(t0, 2 * SEG), :] = (abuf[pl.ds(t0, 2 * SEG), :] + omg * b).astype(BF)
        pltpu.make_async_copy(outbuf.at[pl.ds(t0, 2 * SEG), :],
                              out_hbm.at[pl.ds(t0, 2 * SEG), :], sem_out).start()
        return out_o[:M].astype(BF).astype(F32)

    with jax.named_scope("ph_pair"):
        jax.lax.fori_loop(0, N_PAIRS, pair, mem_ref[...].astype(F32))

    pltpu.make_async_copy(outbuf, out_hbm, sem_out).wait()


@functools.partial(jax.jit, static_argnames=("B_seg_len",))
def pallas_gated_mix__softmax_full_mha__memory_aug_recurrent_mem_tr__prompt_kernel(
    A_x: jax.Array,
    A_wqkv: jax.Array,
    A_wo: jax.Array,
    B_x: jax.Array,
    B_mem0: jax.Array,
    B_Wq: jax.Array,
    B_Wk: jax.Array,
    B_Wv: jax.Array,
    B_Wo: jax.Array,
    B_seg_len: int,
    gate_w: jax.Array,
):
    assert B_seg_len == SEG
    assert A_x.shape == (1, S, D)
    assert B_Wq.shape == (D, HB, DHB) and B_Wo.shape == (HB, DHB, D)

    any_spec = pl.BlockSpec(memory_space=pl.ANY)
    vmem_spec = pl.BlockSpec(memory_space=pltpu.VMEM)
    out = pl.pallas_call(
        _kernel,
        out_shape=jax.ShapeDtypeStruct((S, D), BF),
        in_specs=[any_spec, any_spec, any_spec, vmem_spec, any_spec, any_spec,
                  any_spec, any_spec, vmem_spec],
        out_specs=any_spec,
        scratch_shapes=[
            pltpu.VMEM((S, D), BF),
            pltpu.VMEM((3, D, D), BF),
            pltpu.VMEM((D, D), BF),
            pltpu.VMEM((S, D), BF),
            pltpu.VMEM((D, S), BF),
            pltpu.VMEM((D, S), BF),
            pltpu.VMEM((D, S), BF),
            pltpu.VMEM((S, D), F32),
            pltpu.VMEM((S, 128), F32),
            pltpu.VMEM((D // 2, HB * 384), U32),
            pltpu.VMEM((HB * DHB // 2, D), U32),
            pltpu.VMEM((N_HP * 3, D, 128), U32),
            pltpu.VMEM((S, D), BF),
            pltpu.VMEM((AHEAD, KB, QB), F32),
            pltpu.SemaphoreType.DMA((S // TB + 5,)),
            pltpu.SemaphoreType.DMA((N_HP,)),
            pltpu.SemaphoreType.DMA(()),
        ],
        compiler_params=pltpu.CompilerParams(vmem_limit_bytes=124 * 1024 * 1024),
    )(A_x.reshape(S, D), A_wqkv, A_wo, B_mem0.reshape(M, D),
      B_Wq, B_Wk, B_Wv, B_Wo.reshape(HB * DHB, D), gate_w.reshape(1, D))
    return out.reshape(1, S, D)
```

```python
import functools
import math

import jax
import jax.numpy as jnp
import jax.experimental.pallas as pl
import jax.experimental.pallas.tpu as pltpu

BF = jnp.bfloat16
F32 = jnp.float32
U32 = jnp.uint32

S = 2048
D = 1024
HA, DHA = 32, 32
HB, DHB = 32, 128
M = 8
SEG = 32
L = M + SEG

LOG2E = math.log2(math.e)
CA = DHA ** -0.5 * LOG2E
CB = DHB ** -0.5 * LOG2E
NEG_B = -1e9 * LOG2E

TB = 512
QB = 256
KB = 128
AHEAD = 4
UN = 16
GB = 4
NGB = HB // GB
NQ = S // QB
NK = S // KB
N_UNITS = HA * NQ
N_PAIRS = S // (2 * SEG)
N_HP = HB // 2


def _tree(op, xs):
    xs = list(xs)
    while len(xs) > 1:
        nxt = [op(xs[i], xs[i + 1]) for i in range(0, len(xs) - 1, 2)]
        if len(xs) % 2:
            nxt.append(xs[-1])
        xs = nxt
    return xs[0]


def _kernel(ax_hbm, wqkv_hbm, awo_hbm, mem_ref, bwq_hbm, bwk_hbm, bwv_hbm,
            bwo_hbm, gw_ref, out_hbm,
            ax, wqkv, awo, kbuf, qt, vt, ot, abuf, gbuf, wb, wob, stage, outbuf, scarry,
            sem_in, sem_st, sem_out):
    nblk = S // TB

    def ax_cp(i):
        r0 = pl.multiple_of(i * TB, TB)
        return pltpu.make_async_copy(ax_hbm.at[pl.ds(r0, TB), :], ax.at[pl.ds(r0, TB), :],
                                     sem_in.at[i])

    NC = 4
    CW = D // NC

    def wk_cp(c):
        c0 = pl.multiple_of(c * CW, CW)
        return pltpu.make_async_copy(wqkv_hbm.at[:, pl.ds(D + c0, CW)],
                                     wqkv.at[1, :, pl.ds(c0, CW)], sem_in.at[nblk + 5 + c])

    def wqkv_cp(t):
        return pltpu.make_async_copy(wqkv_hbm.at[:, pl.ds(t * D, D)], wqkv.at[t],
                                     sem_in.at[nblk + t])

    awo_cp = pltpu.make_async_copy(awo_hbm, awo, sem_in.at[nblk + 3])
    wob_cp = pltpu.make_async_copy(bwo_hbm.bitcast(U32), wob, sem_in.at[nblk + 4])

    bw_u32 = [r.bitcast(U32) for r in (bwq_hbm, bwk_hbm, bwv_hbm)]

    def stage_cp(hp, t):
        return pltpu.make_async_copy(bw_u32[t].at[:, hp, :], stage.at[hp * 3 + t],
                                     sem_st.at[hp])

    ax_cp(0).start()
    for c in range(NC):
        wk_cp(c).start()
    for i in range(1, nblk):
        ax_cp(i).start()
    wqkv_cp(0).start()
    wqkv_cp(2).start()

    ax_cp(0).wait()

    def k_proj0(c, carry):
        wk_cp(c).wait()
        c0 = pl.multiple_of(c * CW, CW)
        k = jnp.dot(ax[0:TB, :], wqkv[1, :, pl.ds(c0, CW)], preferred_element_type=F32)
        kbuf[0:TB // 2, pl.ds(c0, CW)] = pltpu.bitcast(k.astype(BF), U32)
        return carry

    def k_proj(i, c):
        ax_cp(i).wait()
        r0 = pl.multiple_of(i * TB, TB)
        rh = pl.multiple_of(i * (TB // 2), TB // 2)
        k = jnp.dot(ax[pl.ds(r0, TB), :], wqkv[1], preferred_element_type=F32)
        kbuf[pl.ds(rh, TB // 2), :] = pltpu.bitcast(k.astype(BF), U32)
        return c

    with jax.named_scope("ph_kproj0"):
        jax.lax.fori_loop(0, NC, k_proj0, 0)
    with jax.named_scope("ph_kproj"):
        jax.lax.fori_loop(1, nblk, k_proj, 0)

    wqkv_cp(0).wait()
    wqkv_cp(2).wait()
    for hp in range(N_HP):
        for t in range(3):
            stage_cp(hp, t).start(priority=1)
    awo_cp.start(priority=1)
    wob_cp.start(priority=1)

    def qv_proj(i, c):
        r0 = pl.multiple_of(i * TB, TB)
        xb = ax[pl.ds(r0, TB), :]
        q = jnp.dot(xb, wqkv[0], preferred_element_type=F32) * CA
        qt[:, pl.ds(r0, TB)] = q.T.astype(BF)
        v = jnp.dot(xb, wqkv[2], preferred_element_type=F32)
        vt[:, pl.ds(r0, TB)] = pltpu.bitcast(v.T.astype(BF), U32)
        z = jnp.sum(xb.astype(F32) * gw_ref[...].astype(F32), axis=1, keepdims=True)
        gbuf[pl.ds(r0, TB), :] = jnp.broadcast_to(1.0 / (1.0 + jnp.exp(-z)), (TB, 128))
        return c

    with jax.named_scope("ph_qvproj"):
        jax.lax.fori_loop(0, nblk, qv_proj, 0)

    def unit_setup(u):
        h = u % HA
        g0 = pl.multiple_of((h // 4) * 128, 128)
        h0 = pl.multiple_of(h * DHA, DHA)
        q0 = pl.multiple_of((u // HA) * QB, QB)
        qg = pltpu.bitcast(qt[pl.ds(g0, 128), pl.ds(q0, QB)], U32)
        rows = jax.lax.broadcasted_iota(jnp.int32, (64, QB), 0)
        qm = pltpu.bitcast(jnp.where(rows // 16 == h % 4, qg, U32(0)), BF)
        return qm, g0, h0, q0

    def qk_chunk(setup, j):
        qm, g0, _, _ = setup
        kb = pltpu.bitcast(kbuf[j * KB // 2:(j + 1) * KB // 2, pl.ds(g0, 128)], BF)
        return jnp.dot(kb, qm, preferred_element_type=F32)

    def attn_iter(it, c):
        setup = [unit_setup(it * UN + k) for k in range(UN)]
        setup_next = unit_setup(jnp.minimum(it * UN + UN, N_UNITS - 1))
        items = [(uu, j) for uu in range(UN) for j in range(NK)]
        n = len(items)
        state = {}

        def pv(i, p, al, l):
            uu, j = items[i]
            _, _, h0, q0 = setup[uu]
            hh0 = pl.multiple_of(h0 // 2, DHA // 2)
            vtb = pltpu.bitcast(vt[pl.ds(hh0, DHA // 2), j * KB:(j + 1) * KB], BF)
            d = jnp.dot(vtb, p, preferred_element_type=F32)
            acc = d if j == 0 else state["acc"] * al + d
            state["acc"] = acc
            if j == NK - 1:
                o = acc / jnp.sum(l, axis=0, keepdims=True)
                ot[pl.ds(h0, DHA), pl.ds(q0, QB)] = o.astype(BF)

        ss = {i: scarry[i] for i in range(AHEAD)}
        m = l = None
        pend = None
        for i, (uu, j) in enumerate(items):
            if i + AHEAD < n:
                uu2, j2 = items[i + AHEAD]
                ss[i + AHEAD] = qk_chunk(setup[uu2], j2)
            else:
                scarry[i + AHEAD - n] = qk_chunk(setup_next, i + AHEAD - n)
            if pend is not None:
                pv(*pend)
            s = ss.pop(i)
            bm = _tree(jnp.maximum, [s[8 * r:8 * r + 8] for r in range(KB // 8)])
            bm = jnp.max(bm, axis=0, keepdims=True)
            if j == 0:
                m, al = bm, None
                p = jnp.exp2(s - m)
                l = _tree(jnp.add, [p[8 * r:8 * r + 8] for r in range(KB // 8)])
            else:
                mn = jnp.maximum(m, bm)
                al = jnp.exp2(m - mn)
                p = jnp.exp2(s - mn)
                l = l * al + _tree(jnp.add, [p[8 * r:8 * r + 8] for r in range(KB // 8)])
                m = mn
            pend = (i, p.astype(BF), al, l)
        pv(*pend)
        return c

    setup0 = unit_setup(0)
    for j in range(AHEAD):
        scarry[j] = qk_chunk(setup0, j)
    with jax.named_scope("ph_attn"):
        jax.lax.fori_loop(0, N_UNITS // UN, attn_iter, 0)

    awo_cp.wait()

    def a_out(i, c):
        r0 = pl.multiple_of(i * TB, TB)
        a = jax.lax.dot_general(ot[:, pl.ds(r0, TB)], awo[...], (((0,), (0,)), ((), ())),
                                preferred_element_type=F32)
        g = gbuf[pl.ds(r0, TB), :]
        abuf[pl.ds(r0, TB), :] = a * jnp.concatenate([g] * (D // 128), axis=1)
        return c

    with jax.named_scope("ph_aout"):
        jax.lax.fori_loop(0, nblk, a_out, 0)

    def relayout(hp, c):
        pltpu.make_async_copy(stage.at[pl.ds(hp * 3, 3)], stage.at[pl.ds(hp * 3, 3)],
                              sem_st.at[hp]).wait()
        for t in range(3):
            ev = stage[hp * 3 + t, pl.ds(0, D // 2, stride=2), :]
            od = stage[hp * 3 + t, pl.ds(1, D // 2, stride=2), :]
            lo = (ev & U32(0xFFFF)) | (od << 16)
            hi = (ev >> 16) | (od & U32(0xFFFF0000))
            c0 = pl.multiple_of(hp * 768 + t * 128, 128)
            wb[:, pl.ds(c0, 128)] = lo
            wb[:, pl.ds(c0 + 384, 128)] = hi
        return c

    with jax.named_scope("ph_relayout"):
        jax.lax.fori_loop(0, N_HP, relayout, 0)

    wob_cp.wait()

    NE, NO = 32, 48
    ri = jax.lax.broadcasted_iota(jnp.int32, (NE, L), 0)
    ci = jax.lax.broadcasted_iota(jnp.int32, (NE, L), 1)
    mask_e = (ri < M) | (ri >= ci)
    fill_e = NEG_B
    ri = jax.lax.broadcasted_iota(jnp.int32, (NO, 2 * L), 0)
    ci = jax.lax.broadcasted_iota(jnp.int32, (NO, 2 * L), 1)
    own = ((ri < L) & (ci >= L)) | ((ri >= L) & (ci < L))
    qi = jnp.where(ri < L, ri, ri - 8)
    ki = jnp.where(ci < L, ci, ci - L)
    mask_o = own & ((qi < M) | (qi >= ki))
    fill_o = jnp.where(own, NEG_B, -3e38)

    def qkv_dot(lhs, g):
        w = pltpu.bitcast(wb[:, g * GB * 384:(g + 1) * GB * 384], BF)
        return jnp.dot(lhs, w, preferred_element_type=F32)

    def qk_dots(qrows, kvrows):
        res = []
        for hh in range(GB):
            b = hh * 384
            q = (qrows[:, b:b + 128] * CB).astype(BF)
            k = kvrows[:, b + 128:b + 256].astype(BF)
            v = kvrows[:, b + 256:b + 384].astype(BF)
            s = jax.lax.dot_general(q, k, (((1,), (1,)), ((), ())), preferred_element_type=F32)
            res.append((s, v))
        return res

    def pv_dots(sv, mask, fill):
        outs = []
        for s, v in sv:
            s = jnp.where(mask, s, fill)
            mx = jnp.max(s, axis=1, keepdims=True)
            p = jnp.exp2(s - mx)
            l = jnp.sum(p, axis=1, keepdims=True)
            o = jnp.dot(p.astype(BF), v, preferred_element_type=F32)
            outs.append(o / l)
        return jnp.concatenate(outs, axis=1)

    def wo_dot(lhs, g):
        w = pltpu.bitcast(wob[g * GB * 64:(g + 1) * GB * 64, :], BF)
        return jnp.dot(lhs.astype(BF), w, preferred_element_type=F32)

    def run_step(lhs, rows_fn, mask, fill):
        qkv, sv, o = {}, {}, {}
        out = None
        qkv[0] = qkv_dot(lhs, 0)
        for g in range(NGB + 2):
            if g + 1 < NGB:
                qkv[g + 1] = qkv_dot(lhs, g + 1)
            if 0 <= g - 1 < NGB:
                o[g - 1] = pv_dots(sv[g - 1], mask, fill)
            if g < NGB:
                sv[g] = qk_dots(*rows_fn(qkv[g], g))
            if 0 <= g - 2 < NGB:
                d = wo_dot(o[g - 2], g - 2)
                out = d if out is None else out + d
        return out, qkv

    def pair(j, mem):
        t0 = pl.multiple_of(j * 2 * SEG, 2 * SEG)
        t1 = pl.multiple_of(j * 2 * SEG + SEG, SEG)
        x_e = ax[pl.ds(t0, 48), :].astype(F32)[:40]
        x_o = ax[pl.ds(t1, SEG), :].astype(F32)[8:]
        lhs_e = jnp.concatenate([mem, x_e], axis=0).astype(BF)
        out_e, qkv_e = run_step(lhs_e, lambda q, g: (q[:NE], q[:L]), mask_e, fill_e)
        mem1 = out_e[:M].astype(BF).astype(F32)
        lhs_o = jnp.concatenate([mem1, x_o], axis=0).astype(BF)

        def rows_o(q, g):
            e = qkv_e[g]
            seg_o = [q[:8], e[40:48], q[8:32]]
            return (jnp.concatenate(seg_o + [e[32:40]], axis=0),
                    jnp.concatenate([e[:L]] + seg_o, axis=0))

        out_o, _ = run_step(lhs_o, rows_o, mask_o, fill_o)
        b = jnp.concatenate([out_e[8:32], out_o[40:48], out_o[8:40]], axis=0)
        g = gbuf[pl.ds(t0, 2 * SEG), :]
        omg = jnp.concatenate([1.0 - g] * (D // 128), axis=1)
        outbuf[pl.ds(t0, 2 * SEG), :] = (abuf[pl.ds(t0, 2 * SEG), :] + omg * b).astype(BF)
        pltpu.make_async_copy(outbuf.at[pl.ds(t0, 2 * SEG), :],
                              out_hbm.at[pl.ds(t0, 2 * SEG), :], sem_out).start()
        return out_o[:M].astype(BF).astype(F32)

    with jax.named_scope("ph_pair"):
        jax.lax.fori_loop(0, N_PAIRS, pair, mem_ref[...].astype(F32))

    pltpu.make_async_copy(outbuf, out_hbm, sem_out).wait()


@functools.partial(jax.jit, static_argnames=("B_seg_len",))
def pallas_gated_mix__softmax_full_mha__memory_aug_recurrent_mem_tr__prompt_kernel(
    A_x: jax.Array,
    A_wqkv: jax.Array,
    A_wo: jax.Array,
    B_x: jax.Array,
    B_mem0: jax.Array,
    B_Wq: jax.Array,
    B_Wk: jax.Array,
    B_Wv: jax.Array,
    B_Wo: jax.Array,
    B_seg_len: int,
    gate_w: jax.Array,
):
    assert B_seg_len == SEG
    assert A_x.shape == (1, S, D)
    assert B_Wq.shape == (D, HB, DHB) and B_Wo.shape == (HB, DHB, D)

    any_spec = pl.BlockSpec(memory_space=pl.ANY)
    vmem_spec = pl.BlockSpec(memory_space=pltpu.VMEM)
    out = pl.pallas_call(
        _kernel,
        out_shape=jax.ShapeDtypeStruct((S, D), BF),
        in_specs=[any_spec, any_spec, any_spec, vmem_spec, any_spec, any_spec,
                  any_spec, any_spec, vmem_spec],
        out_specs=any_spec,
        scratch_shapes=[
            pltpu.VMEM((S, D), BF),
            pltpu.VMEM((3, D, D), BF),
            pltpu.VMEM((D, D), BF),
            pltpu.VMEM((S // 2, D), U32),
            pltpu.VMEM((D, S), BF),
            pltpu.VMEM((D // 2, S), U32),
            pltpu.VMEM((D, S), BF),
            pltpu.VMEM((S, D), F32),
            pltpu.VMEM((S, 128), F32),
            pltpu.VMEM((D // 2, HB * 384), U32),
            pltpu.VMEM((HB * DHB // 2, D), U32),
            pltpu.VMEM((N_HP * 3, D, 128), U32),
            pltpu.VMEM((S, D), BF),
            pltpu.VMEM((AHEAD, KB, QB), F32),
            pltpu.SemaphoreType.DMA((S // TB + 9,)),
            pltpu.SemaphoreType.DMA((N_HP,)),
            pltpu.SemaphoreType.DMA(()),
        ],
        compiler_params=pltpu.CompilerParams(vmem_limit_bytes=124 * 1024 * 1024),
    )(A_x.reshape(S, D), A_wqkv, A_wo, B_mem0.reshape(M, D),
      B_Wq, B_Wk, B_Wv, B_Wo.reshape(HB * DHB, D), gate_w.reshape(1, D))
    return out.reshape(1, S, D)
```

```python
import functools
import math

import jax
import jax.numpy as jnp
import jax.experimental.pallas as pl
import jax.experimental.pallas.tpu as pltpu

BF = jnp.bfloat16
F32 = jnp.float32
U32 = jnp.uint32

S = 2048
D = 1024
HA, DHA = 32, 32
HB, DHB = 32, 128
M = 8
SEG = 32
L = M + SEG

LOG2E = math.log2(math.e)
CA = DHA ** -0.5 * LOG2E
CB = DHB ** -0.5 * LOG2E
NEG_B = -1e9 * LOG2E

TB = 512
QB = 256
KB = 128
AHEAD = 4
UN = 16
GB = 4
NGB = HB // GB
NQ = S // QB
NK = S // KB
N_UNITS = HA * NQ
N_PAIRS = S // (2 * SEG)
N_HP = HB // 2


def _tree(op, xs):
    xs = list(xs)
    while len(xs) > 1:
        nxt = [op(xs[i], xs[i + 1]) for i in range(0, len(xs) - 1, 2)]
        if len(xs) % 2:
            nxt.append(xs[-1])
        xs = nxt
    return xs[0]


def _kernel(ax_hbm, wqkv_hbm, awo_hbm, mem_ref, bwq_hbm, bwk_hbm, bwv_hbm,
            bwo_hbm, gw_ref, out_hbm,
            ax, wqkv, awo, kbuf, qt, vt, ot, abuf, gbuf, wb, wob, stage, outbuf, scarry, spare_idx,
            sem_in, sem_st, sem_out):
    nblk = S // TB

    def ax_cp(i):
        r0 = pl.multiple_of(i * TB, TB)
        return pltpu.make_async_copy(ax_hbm.at[pl.ds(r0, TB), :], ax.at[pl.ds(r0, TB), :],
                                     sem_in.at[i])

    wqkv_u32 = wqkv_hbm.bitcast(U32)
    NC = 4
    CW = D // NC

    def wk_cp(c):
        c0 = pl.multiple_of(c * CW, CW)
        return pltpu.make_async_copy(wqkv_u32.at[:, pl.ds(D + c0, CW)],
                                     wqkv.at[1, :, pl.ds(c0, CW)], sem_in.at[nblk + 5 + c])

    def wqkv_cp(t):
        return pltpu.make_async_copy(wqkv_u32.at[:, pl.ds(t * D, D)], wqkv.at[t],
                                     sem_in.at[nblk + t])

    awo_cp = pltpu.make_async_copy(awo_hbm.bitcast(U32), awo, sem_in.at[nblk + 3])
    wob_cp = pltpu.make_async_copy(bwo_hbm.bitcast(U32), wob, sem_in.at[nblk + 4])

    bw_u32 = [r.bitcast(U32) for r in (bwq_hbm, bwk_hbm, bwv_hbm)]

    def stage_cp(hp, t):
        return pltpu.make_async_copy(bw_u32[t].at[:, hp, :], stage.at[hp * 3 + t],
                                     sem_st.at[hp])

    spare_idx[0] = N_HP * 3
    ax_cp(0).start()
    for c in range(NC):
        wk_cp(c).start()
    for i in range(1, nblk):
        ax_cp(i).start()
    wqkv_cp(0).start()
    wqkv_cp(2).start()

    ax_cp(0).wait()

    def k_proj0(c, carry):
        wk_cp(c).wait()
        c0 = pl.multiple_of(c * CW, CW)
        k = jnp.dot(ax[0:TB, :], pltpu.bitcast(wqkv[1, :, pl.ds(c0, CW)], BF),
                    preferred_element_type=F32)
        kbuf[0:TB // 2, pl.ds(c0, CW)] = pltpu.bitcast(k.astype(BF), U32)
        return carry

    def k_proj(i, c):
        ax_cp(i).wait()
        r0 = pl.multiple_of(i * TB, TB)
        rh = pl.multiple_of(i * (TB // 2), TB // 2)
        k = jnp.dot(ax[pl.ds(r0, TB), :], pltpu.bitcast(wqkv[1], BF), preferred_element_type=F32)
        kbuf[pl.ds(rh, TB // 2), :] = pltpu.bitcast(k.astype(BF), U32)
        return c

    with jax.named_scope("ph_kproj0"):
        jax.lax.fori_loop(0, NC, k_proj0, 0)
    with jax.named_scope("ph_kproj"):
        jax.lax.fori_loop(1, nblk, k_proj, 0)

    wqkv_cp(0).wait()
    wqkv_cp(2).wait()
    for hp in range(N_HP):
        for t in range(3):
            stage_cp(hp, t).start(priority=1)
    awo_cp.start(priority=1)
    wob_cp.start(priority=1)

    def qv_proj(i, c):
        r0 = pl.multiple_of(i * TB, TB)
        xb = ax[pl.ds(r0, TB), :]
        q = jnp.dot(xb, pltpu.bitcast(wqkv[0], BF), preferred_element_type=F32) * CA
        qt[:, pl.ds(r0, TB)] = q.T.astype(BF)
        v = jnp.dot(xb, pltpu.bitcast(wqkv[2], BF), preferred_element_type=F32)
        vt[:, pl.ds(r0, TB)] = pltpu.bitcast(v.T.astype(BF), U32)
        z = jnp.sum(xb.astype(F32) * gw_ref[...].astype(F32), axis=1, keepdims=True)
        gbuf[pl.ds(r0, TB), :] = jnp.broadcast_to(1.0 / (1.0 + jnp.exp(-z)), (TB, 128))
        return c

    with jax.named_scope("ph_qvproj"):
        jax.lax.fori_loop(0, nblk, qv_proj, 0)

    def unit_setup(u):
        h = u % HA
        g0 = pl.multiple_of((h // 4) * 128, 128)
        h0 = pl.multiple_of(h * DHA, DHA)
        q0 = pl.multiple_of((u // HA) * QB, QB)
        qg = pltpu.bitcast(qt[pl.ds(g0, 128), pl.ds(q0, QB)], U32)
        rows = jax.lax.broadcasted_iota(jnp.int32, (64, QB), 0)
        qm = pltpu.bitcast(jnp.where(rows // 16 == h % 4, qg, U32(0)), BF)
        return qm, g0, h0, q0

    def qk_chunk(setup, j):
        qm, g0, _, _ = setup
        kb = pltpu.bitcast(kbuf[j * KB // 2:(j + 1) * KB // 2, pl.ds(g0, 128)], BF)
        return jnp.dot(kb, qm, preferred_element_type=F32)

    def attn_iter(it, c):
        setup = [unit_setup(it * UN + k) for k in range(UN)]
        setup_next = unit_setup(jnp.minimum(it * UN + UN, N_UNITS - 1))
        items = [(uu, j) for uu in range(UN) for j in range(NK)]
        n = len(items)
        state = {}

        def pv(i, p, al, l):
            uu, j = items[i]
            _, _, h0, q0 = setup[uu]
            hh0 = pl.multiple_of(h0 // 2, DHA // 2)
            vtb = pltpu.bitcast(vt[pl.ds(hh0, DHA // 2), j * KB:(j + 1) * KB], BF)
            d = jnp.dot(vtb, p, preferred_element_type=F32)
            acc = d if j == 0 else state["acc"] * al + d
            state["acc"] = acc
            if j == NK - 1:
                o = acc / jnp.sum(l, axis=0, keepdims=True)
                ot[pl.ds(h0, DHA), pl.ds(q0, QB)] = o.astype(BF)

        ss = {i: scarry[i] for i in range(AHEAD)}
        m = l = None
        pend = None
        for i, (uu, j) in enumerate(items):
            if i + AHEAD < n:
                uu2, j2 = items[i + AHEAD]
                ss[i + AHEAD] = qk_chunk(setup[uu2], j2)
            else:
                scarry[i + AHEAD - n] = qk_chunk(setup_next, i + AHEAD - n)
            if pend is not None:
                pv(*pend)
            s = ss.pop(i)
            bm = _tree(jnp.maximum, [s[8 * r:8 * r + 8] for r in range(KB // 8)])
            bm = jnp.max(bm, axis=0, keepdims=True)
            if j == 0:
                m, al = bm, None
                p = jnp.exp2(s - m)
                l = _tree(jnp.add, [p[8 * r:8 * r + 8] for r in range(KB // 8)])
            else:
                mn = jnp.maximum(m, bm)
                al = jnp.exp2(m - mn)
                p = jnp.exp2(s - mn)
                l = l * al + _tree(jnp.add, [p[8 * r:8 * r + 8] for r in range(KB // 8)])
                m = mn
            pend = (i, p.astype(BF), al, l)
        pv(*pend)
        return c

    setup0 = unit_setup(0)
    for j in range(AHEAD):
        scarry[j] = qk_chunk(setup0, j)
    with jax.named_scope("ph_attn"):
        jax.lax.fori_loop(0, N_UNITS // UN, attn_iter, 0)

    awo_cp.wait()
    for hp in range(N_HP):
        pltpu.make_async_copy(stage.at[pl.ds(hp * 3, 3)], stage.at[pl.ds(hp * 3, 3)],
                              sem_st.at[hp]).wait()

    RS, CS, SUB = 4, 8, 8
    HP_IT = N_HP // nblk

    def relayout(hp, t, sub):
        nr = D // 2 // SUB
        ev = stage[hp * 3 + t, pl.ds(2 * sub * nr, nr, stride=2), :]
        od = stage[hp * 3 + t, pl.ds(2 * sub * nr + 1, nr, stride=2), :]
        lo = (ev & U32(0xFFFF)) | (od << 16)
        hi = (ev >> 16) | (od & U32(0xFFFF0000))
        c0 = pl.multiple_of(hp * 768 + t * 128, 128)
        wb[sub * nr:(sub + 1) * nr, pl.ds(c0, 128)] = lo
        wb[sub * nr:(sub + 1) * nr, pl.ds(c0 + 384, 128)] = hi

    def a_out(i, c):
        r0 = pl.multiple_of(i * TB, TB)
        lhs = ot[:, pl.ds(r0, TB)].T
        pieces = [(i * HP_IT + k, t, sub) for k in range(HP_IT) for t in range(3)
                  for sub in range(SUB)]
        slots = [(cc, rr) for cc in range(CS) for rr in range(RS)]
        spare = spare_idx[0]
        rb, cw = TB // RS, D // CS
        for si, (cc, rr) in enumerate(slots):
            a = jnp.dot(lhs[rr * rb:(rr + 1) * rb], pltpu.bitcast(awo[:, cc * cw:(cc + 1) * cw], BF),
                        preferred_element_type=F32)
            rows = pl.ds(pl.multiple_of(r0 + rr * rb, rb), rb)
            abuf[rows, cc * cw:(cc + 1) * cw] = a * gbuf[rows, :]
            stage[spare, 0:8, :] = pltpu.bitcast(a[0:8], U32)
            for q, p in enumerate(pieces):
                if q * len(slots) // len(pieces) == si:
                    relayout(*p)
        return c

    with jax.named_scope("ph_aout"):
        jax.lax.fori_loop(0, nblk, a_out, 0)

    wob_cp.wait()

    NE, NO = 32, 48
    ri = jax.lax.broadcasted_iota(jnp.int32, (NE, L), 0)
    ci = jax.lax.broadcasted_iota(jnp.int32, (NE, L), 1)
    mask_e = (ri < M) | (ri >= ci)
    fill_e = NEG_B
    ri = jax.lax.broadcasted_iota(jnp.int32, (NO, 2 * L), 0)
    ci = jax.lax.broadcasted_iota(jnp.int32, (NO, 2 * L), 1)
    own = ((ri < L) & (ci >= L)) | ((ri >= L) & (ci < L))
    qi = jnp.where(ri < L, ri, ri - 8)
    ki = jnp.where(ci < L, ci, ci - L)
    mask_o = own & ((qi < M) | (qi >= ki))
    fill_o = jnp.where(own, NEG_B, -3e38)

    def qkv_dot(lhs, g):
        w = pltpu.bitcast(wb[:, g * GB * 384:(g + 1) * GB * 384], BF)
        return jnp.dot(lhs, w, preferred_element_type=F32)

    def qk_dots(qrows, kvrows):
        res = []
        for hh in range(GB):
            b = hh * 384
            q = (qrows[:, b:b + 128] * CB).astype(BF)
            k = kvrows[:, b + 128:b + 256].astype(BF)
            v = kvrows[:, b + 256:b + 384].astype(BF)
            s = jax.lax.dot_general(q, k, (((1,), (1,)), ((), ())), preferred_element_type=F32)
            res.append((s, v))
        return res

    def pv_dots(sv, mask, fill):
        outs = []
        for s, v in sv:
            s = jnp.where(mask, s, fill)
            mx = jnp.max(s, axis=1, keepdims=True)
            p = jnp.exp2(s - mx)
            l = jnp.sum(p, axis=1, keepdims=True)
            o = jnp.dot(p.astype(BF), v, preferred_element_type=F32)
            outs.append(o / l)
        return jnp.concatenate(outs, axis=1)

    def wo_dot(lhs, g):
        w = pltpu.bitcast(wob[g * GB * 64:(g + 1) * GB * 64, :], BF)
        return jnp.dot(lhs.astype(BF), w, preferred_element_type=F32)

    def run_step(lhs, rows_fn, mask, fill):
        qkv, sv, o = {}, {}, {}
        out = None
        qkv[0] = qkv_dot(lhs, 0)
        for g in range(NGB + 2):
            if g + 1 < NGB:
                qkv[g + 1] = qkv_dot(lhs, g + 1)
            if 0 <= g - 1 < NGB:
                o[g - 1] = pv_dots(sv[g - 1], mask, fill)
            if g < NGB:
                sv[g] = qk_dots(*rows_fn(qkv[g], g))
            if 0 <= g - 2 < NGB:
                d = wo_dot(o[g - 2], g - 2)
                out = d if out is None else out + d
        return out, qkv

    def pair(j, mem):
        t0 = pl.multiple_of(j * 2 * SEG, 2 * SEG)
        t1 = pl.multiple_of(j * 2 * SEG + SEG, SEG)
        x_e = ax[pl.ds(t0, 48), :].astype(F32)[:40]
        x_o = ax[pl.ds(t1, SEG), :].astype(F32)[8:]
        lhs_e = jnp.concatenate([mem, x_e], axis=0).astype(BF)
        out_e, qkv_e = run_step(lhs_e, lambda q, g: (q[:NE], q[:L]), mask_e, fill_e)
        mem1 = out_e[:M].astype(BF).astype(F32)
        lhs_o = jnp.concatenate([mem1, x_o], axis=0).astype(BF)

        def rows_o(q, g):
            e = qkv_e[g]
            seg_o = [q[:8], e[40:48], q[8:32]]
            return (jnp.concatenate(seg_o + [e[32:40]], axis=0),
                    jnp.concatenate([e[:L]] + seg_o, axis=0))

        out_o, _ = run_step(lhs_o, rows_o, mask_o, fill_o)
        b = jnp.concatenate([out_e[8:32], out_o[40:48], out_o[8:40]], axis=0)
        g = gbuf[pl.ds(t0, 2 * SEG), :]
        omg = jnp.concatenate([1.0 - g] * (D // 128), axis=1)
        outbuf[pl.ds(t0, 2 * SEG), :] = (abuf[pl.ds(t0, 2 * SEG), :] + omg * b).astype(BF)
        pltpu.make_async_copy(outbuf.at[pl.ds(t0, 2 * SEG), :],
                              out_hbm.at[pl.ds(t0, 2 * SEG), :], sem_out).start()
        return out_o[:M].astype(BF).astype(F32)

    with jax.named_scope("ph_pair"):
        jax.lax.fori_loop(0, N_PAIRS, pair, mem_ref[...].astype(F32))

    pltpu.make_async_copy(outbuf, out_hbm, sem_out).wait()


@functools.partial(jax.jit, static_argnames=("B_seg_len",))
def pallas_gated_mix__softmax_full_mha__memory_aug_recurrent_mem_tr__prompt_kernel(
    A_x: jax.Array,
    A_wqkv: jax.Array,
    A_wo: jax.Array,
    B_x: jax.Array,
    B_mem0: jax.Array,
    B_Wq: jax.Array,
    B_Wk: jax.Array,
    B_Wv: jax.Array,
    B_Wo: jax.Array,
    B_seg_len: int,
    gate_w: jax.Array,
):
    assert B_seg_len == SEG
    assert A_x.shape == (1, S, D)
    assert B_Wq.shape == (D, HB, DHB) and B_Wo.shape == (HB, DHB, D)

    any_spec = pl.BlockSpec(memory_space=pl.ANY)
    vmem_spec = pl.BlockSpec(memory_space=pltpu.VMEM)
    out = pl.pallas_call(
        _kernel,
        out_shape=jax.ShapeDtypeStruct((S, D), BF),
        in_specs=[any_spec, any_spec, any_spec, vmem_spec, any_spec, any_spec,
                  any_spec, any_spec, vmem_spec],
        out_specs=any_spec,
        scratch_shapes=[
            pltpu.VMEM((S, D), BF),
            pltpu.VMEM((3, D // 2, D), U32),
            pltpu.VMEM((D // 2, D), U32),
            pltpu.VMEM((S // 2, D), U32),
            pltpu.VMEM((D, S), BF),
            pltpu.VMEM((D // 2, S), U32),
            pltpu.VMEM((D, S), BF),
            pltpu.VMEM((S, D), F32),
            pltpu.VMEM((S, 128), F32),
            pltpu.VMEM((D // 2, HB * 384), U32),
            pltpu.VMEM((HB * DHB // 2, D), U32),
            pltpu.VMEM((N_HP * 3 + 1, D, 128), U32),
            pltpu.VMEM((S, D), BF),
            pltpu.VMEM((AHEAD, KB, QB), F32),
            pltpu.SMEM((1,), jnp.int32),
            pltpu.SemaphoreType.DMA((S // TB + 9,)),
            pltpu.SemaphoreType.DMA((N_HP,)),
            pltpu.SemaphoreType.DMA(()),
        ],
        compiler_params=pltpu.CompilerParams(vmem_limit_bytes=124 * 1024 * 1024),
    )(A_x.reshape(S, D), A_wqkv, A_wo, B_mem0.reshape(M, D),
      B_Wq, B_Wk, B_Wv, B_Wo.reshape(HB * DHB, D), gate_w.reshape(1, D))
    return out.reshape(1, S, D)
```

```python
import functools
import math

import jax
import jax.numpy as jnp
import jax.experimental.pallas as pl
import jax.experimental.pallas.tpu as pltpu

BF = jnp.bfloat16
F32 = jnp.float32
U32 = jnp.uint32

S = 2048
D = 1024
HA, DHA = 32, 32
HB, DHB = 32, 128
M = 8
SEG = 32
L = M + SEG

LOG2E = math.log2(math.e)
CA = DHA ** -0.5 * LOG2E
CB = DHB ** -0.5 * LOG2E
NEG_B = -1e9 * LOG2E

TB = 512
QB = 256
KB = 128
AHEAD = 4
UN = 16
GB = 4
NGB = HB // GB
NQ = S // QB
NK = S // KB
N_UNITS = HA * NQ
N_PAIRS = S // (2 * SEG)
N_HP = HB // 2


def _tree(op, xs):
    xs = list(xs)
    while len(xs) > 1:
        nxt = [op(xs[i], xs[i + 1]) for i in range(0, len(xs) - 1, 2)]
        if len(xs) % 2:
            nxt.append(xs[-1])
        xs = nxt
    return xs[0]


def _kernel(ax_hbm, wqkv_hbm, awo_hbm, mem_ref, bwq_hbm, bwk_hbm, bwv_hbm,
            bwo_hbm, gw_ref, out_hbm,
            ax, wqkv, awo, kbuf, qt, vt, ot, abuf, gbuf, wb, wob, stage, outbuf, scarry, spare_idx,
            sem_in, sem_st, sem_out):
    nblk = S // TB

    def ax_cp(i):
        r0 = pl.multiple_of(i * TB, TB)
        return pltpu.make_async_copy(ax_hbm.at[pl.ds(r0, TB), :], ax.at[pl.ds(r0, TB), :],
                                     sem_in.at[i])

    wqkv_u32 = wqkv_hbm.bitcast(U32)
    NC = 4
    CW = D // NC

    def wk_cp(c):
        c0 = pl.multiple_of(c * CW, CW)
        return pltpu.make_async_copy(wqkv_u32.at[:, pl.ds(D + c0, CW)],
                                     wqkv.at[1, :, pl.ds(c0, CW)], sem_in.at[nblk + 5 + c])

    def wqkv_cp(t):
        return pltpu.make_async_copy(wqkv_u32.at[:, pl.ds(t * D, D)], wqkv.at[t],
                                     sem_in.at[nblk + t])

    awo_cp = pltpu.make_async_copy(awo_hbm.bitcast(U32), awo, sem_in.at[nblk + 3])
    wob_cp = pltpu.make_async_copy(bwo_hbm.bitcast(U32), wob, sem_in.at[nblk + 4])

    bw_u32 = [r.bitcast(U32) for r in (bwq_hbm, bwk_hbm, bwv_hbm)]

    def stage_cp(hp, t):
        return pltpu.make_async_copy(bw_u32[t].at[:, hp, :], stage.at[hp * 3 + t],
                                     sem_st.at[hp])

    spare_idx[0] = N_HP * 3
    ax_cp(0).start()
    for c in range(NC):
        wk_cp(c).start()
    for i in range(1, nblk):
        ax_cp(i).start()
    wqkv_cp(0).start()
    wqkv_cp(2).start()

    ax_cp(0).wait()

    def k_proj0(c, carry):
        wk_cp(c).wait()
        c0 = pl.multiple_of(c * CW, CW)
        k = jnp.dot(ax[0:TB, :], pltpu.bitcast(wqkv[1, :, pl.ds(c0, CW)], BF),
                    preferred_element_type=F32)
        kbuf[0:TB // 2, pl.ds(c0, CW)] = pltpu.bitcast(k.astype(BF), U32)
        return carry

    def k_proj(i, c):
        ax_cp(i).wait()
        r0 = pl.multiple_of(i * TB, TB)
        rh = pl.multiple_of(i * (TB // 2), TB // 2)
        k = jnp.dot(ax[pl.ds(r0, TB), :], pltpu.bitcast(wqkv[1], BF), preferred_element_type=F32)
        kbuf[pl.ds(rh, TB // 2), :] = pltpu.bitcast(k.astype(BF), U32)
        return c

    with jax.named_scope("ph_kproj0"):
        jax.lax.fori_loop(0, NC, k_proj0, 0)
    with jax.named_scope("ph_kproj"):
        jax.lax.fori_loop(1, nblk, k_proj, 0)

    wqkv_cp(0).wait()
    wqkv_cp(2).wait()
    for hp in range(N_HP):
        for t in range(3):
            stage_cp(hp, t).start(priority=1)
    awo_cp.start(priority=1)
    wob_cp.start(priority=1)

    def qv_proj(i, c):
        r0 = pl.multiple_of(i * TB, TB)
        xb = ax[pl.ds(r0, TB), :]
        q = jnp.dot(xb, pltpu.bitcast(wqkv[0], BF), preferred_element_type=F32) * CA
        qt[:, pl.ds(r0, TB)] = q.T.astype(BF)
        v = jnp.dot(xb, pltpu.bitcast(wqkv[2], BF), preferred_element_type=F32)
        vt[:, pl.ds(r0, TB)] = pltpu.bitcast(v.T.astype(BF), U32)
        z = jnp.sum(xb.astype(F32) * gw_ref[...].astype(F32).reshape(1, D), axis=1, keepdims=True)
        gbuf[pl.ds(r0, TB), :] = jnp.broadcast_to(1.0 / (1.0 + jnp.exp(-z)), (TB, 128))
        return c

    with jax.named_scope("ph_qvproj"):
        jax.lax.fori_loop(0, nblk, qv_proj, 0)

    def unit_setup(u):
        h = u % HA
        g0 = pl.multiple_of((h // 4) * 128, 128)
        h0 = pl.multiple_of(h * DHA, DHA)
        q0 = pl.multiple_of((u // HA) * QB, QB)
        qg = pltpu.bitcast(qt[pl.ds(g0, 128), pl.ds(q0, QB)], U32)
        rows = jax.lax.broadcasted_iota(jnp.int32, (64, QB), 0)
        qm = pltpu.bitcast(jnp.where(rows // 16 == h % 4, qg, U32(0)), BF)
        return qm, g0, h0, q0

    def qk_chunk(setup, j):
        qm, g0, _, _ = setup
        kb = pltpu.bitcast(kbuf[j * KB // 2:(j + 1) * KB // 2, pl.ds(g0, 128)], BF)
        return jnp.dot(kb, qm, preferred_element_type=F32)

    def attn_iter(it, c):
        setup = [unit_setup(it * UN + k) for k in range(UN)]
        setup_next = unit_setup(jnp.minimum(it * UN + UN, N_UNITS - 1))
        items = [(uu, j) for uu in range(UN) for j in range(NK)]
        n = len(items)
        state = {}

        def pv(i, p, al, l):
            uu, j = items[i]
            _, _, h0, q0 = setup[uu]
            hh0 = pl.multiple_of(h0 // 2, DHA // 2)
            vtb = pltpu.bitcast(vt[pl.ds(hh0, DHA // 2), j * KB:(j + 1) * KB], BF)
            d = jnp.dot(vtb, p, preferred_element_type=F32)
            acc = d if j == 0 else state["acc"] * al + d
            state["acc"] = acc
            if j == NK - 1:
                o = acc / jnp.sum(l, axis=0, keepdims=True)
                ot[pl.ds(h0, DHA), pl.ds(q0, QB)] = o.astype(BF)

        ss = {i: scarry[i] for i in range(AHEAD)}
        m = l = None
        pend = None
        for i, (uu, j) in enumerate(items):
            if i + AHEAD < n:
                uu2, j2 = items[i + AHEAD]
                ss[i + AHEAD] = qk_chunk(setup[uu2], j2)
            else:
                scarry[i + AHEAD - n] = qk_chunk(setup_next, i + AHEAD - n)
            if pend is not None:
                pv(*pend)
            s = ss.pop(i)
            bm = _tree(jnp.maximum, [s[8 * r:8 * r + 8] for r in range(KB // 8)])
            bm = jnp.max(bm, axis=0, keepdims=True)
            if j == 0:
                m, al = bm, None
                p = jnp.exp2(s - m)
                l = _tree(jnp.add, [p[8 * r:8 * r + 8] for r in range(KB // 8)])
            else:
                mn = jnp.maximum(m, bm)
                al = jnp.exp2(m - mn)
                p = jnp.exp2(s - mn)
                l = l * al + _tree(jnp.add, [p[8 * r:8 * r + 8] for r in range(KB // 8)])
                m = mn
            pend = (i, p.astype(BF), al, l)
        pv(*pend)
        return c

    setup0 = unit_setup(0)
    for j in range(AHEAD):
        scarry[j] = qk_chunk(setup0, j)
    with jax.named_scope("ph_attn"):
        jax.lax.fori_loop(0, N_UNITS // UN, attn_iter, 0)

    awo_cp.wait()
    for hp in range(N_HP):
        pltpu.make_async_copy(stage.at[pl.ds(hp * 3, 3)], stage.at[pl.ds(hp * 3, 3)],
                              sem_st.at[hp]).wait()

    RS, CS, SUB = 4, 8, 32
    HP_IT = N_HP // nblk

    def relayout(hp, t, sub):
        nr = D // 2 // SUB
        ev = stage[hp * 3 + t, pl.ds(2 * sub * nr, nr, stride=2), :]
        od = stage[hp * 3 + t, pl.ds(2 * sub * nr + 1, nr, stride=2), :]
        lo = (ev & U32(0xFFFF)) | (od << 16)
        hi = (ev >> 16) | (od & U32(0xFFFF0000))
        c0 = pl.multiple_of(hp * 768 + t * 128, 128)
        wb[sub * nr:(sub + 1) * nr, pl.ds(c0, 128)] = lo
        wb[sub * nr:(sub + 1) * nr, pl.ds(c0 + 384, 128)] = hi

    def a_out(i, c):
        r0 = pl.multiple_of(i * TB, TB)
        lhs = ot[:, pl.ds(r0, TB)].T
        pieces = [(i * HP_IT + k, t, sub) for k in range(HP_IT) for t in range(3)
                  for sub in range(SUB)]
        slots = [(cc, rr) for cc in range(CS) for rr in range(RS)]
        spare = spare_idx[0]
        rb, cw = TB // RS, D // CS
        for si, (cc, rr) in enumerate(slots):
            a = jnp.dot(lhs[rr * rb:(rr + 1) * rb], pltpu.bitcast(awo[:, cc * cw:(cc + 1) * cw], BF),
                        preferred_element_type=F32)
            rows = pl.ds(pl.multiple_of(r0 + rr * rb, rb), rb)
            abuf[rows, cc * cw:(cc + 1) * cw] = a * gbuf[rows, :]
            stage[spare, 0:8, :] = pltpu.bitcast(a[0:8, 0:128], U32)
            for q, p in enumerate(pieces):
                if q * len(slots) // len(pieces) == si:
                    relayout(*p)
        return c

    with jax.named_scope("ph_aout"):
        jax.lax.fori_loop(0, nblk, a_out, 0)

    wob_cp.wait()

    NE, NO = 32, 48
    ri = jax.lax.broadcasted_iota(jnp.int32, (NE, L), 0)
    ci = jax.lax.broadcasted_iota(jnp.int32, (NE, L), 1)
    mask_e = (ri < M) | (ri >= ci)
    fill_e = NEG_B
    ri = jax.lax.broadcasted_iota(jnp.int32, (NO, 2 * L), 0)
    ci = jax.lax.broadcasted_iota(jnp.int32, (NO, 2 * L), 1)
    own = ((ri < L) & (ci >= L)) | ((ri >= L) & (ci < L))
    qi = jnp.where(ri < L, ri, ri - 8)
    ki = jnp.where(ci < L, ci, ci - L)
    mask_o = own & ((qi < M) | (qi >= ki))
    fill_o = jnp.where(own, NEG_B, -3e38)

    def qkv_dot(lhs, g):
        w = pltpu.bitcast(wb[:, g * GB * 384:(g + 1) * GB * 384], BF)
        return jnp.dot(lhs, w, preferred_element_type=F32)

    def qk_dots(qrows, kvrows):
        res = []
        for hh in range(GB):
            b = hh * 384
            q = (qrows[:, b:b + 128] * CB).astype(BF)
            k = kvrows[:, b + 128:b + 256].astype(BF)
            v = kvrows[:, b + 256:b + 384].astype(BF)
            s = jax.lax.dot_general(q, k, (((1,), (1,)), ((), ())), preferred_element_type=F32)
            res.append((s, v))
        return res

    def pv_dots(sv, mask, fill):
        outs = []
        for s, v in sv:
            s = jnp.where(mask, s, fill)
            mx = jnp.max(s, axis=1, keepdims=True)
            p = jnp.exp2(s - mx)
            l = jnp.sum(p, axis=1, keepdims=True)
            o = jnp.dot(p.astype(BF), v, preferred_element_type=F32)
            outs.append(o / l)
        return jnp.concatenate(outs, axis=1)

    def wo_dot(lhs, g):
        w = pltpu.bitcast(wob[g * GB * 64:(g + 1) * GB * 64, :], BF)
        return jnp.dot(lhs.astype(BF), w, preferred_element_type=F32)

    def run_step(lhs, rows_fn, mask, fill):
        qkv, sv, o = {}, {}, {}
        out = None
        qkv[0] = qkv_dot(lhs, 0)
        for g in range(NGB + 2):
            if g + 1 < NGB:
                qkv[g + 1] = qkv_dot(lhs, g + 1)
            if 0 <= g - 1 < NGB:
                o[g - 1] = pv_dots(sv[g - 1], mask, fill)
            if g < NGB:
                sv[g] = qk_dots(*rows_fn(qkv[g], g))
            if 0 <= g - 2 < NGB:
                d = wo_dot(o[g - 2], g - 2)
                out = d if out is None else out + d
        return out, qkv

    def pair(j, mem):
        t0 = pl.multiple_of(j * 2 * SEG, 2 * SEG)
        t1 = pl.multiple_of(j * 2 * SEG + SEG, SEG)
        x_e = ax[pl.ds(t0, 48), :].astype(F32)[:40]
        x_o = ax[pl.ds(t1, SEG), :].astype(F32)[8:]
        lhs_e = jnp.concatenate([mem, x_e], axis=0).astype(BF)
        out_e, qkv_e = run_step(lhs_e, lambda q, g: (q[:NE], q[:L]), mask_e, fill_e)
        mem1 = out_e[:M].astype(BF).astype(F32)
        lhs_o = jnp.concatenate([mem1, x_o], axis=0).astype(BF)

        def rows_o(q, g):
            e = qkv_e[g]
            seg_o = [q[:8], e[40:48], q[8:32]]
            return (jnp.concatenate(seg_o + [e[32:40]], axis=0),
                    jnp.concatenate([e[:L]] + seg_o, axis=0))

        out_o, _ = run_step(lhs_o, rows_o, mask_o, fill_o)
        b = jnp.concatenate([out_e[8:32], out_o[40:48], out_o[8:40]], axis=0)
        rows = pl.ds(t0, 2 * SEG)
        omg = jnp.concatenate([1.0 - gbuf[rows, :]] * (D // 128), axis=1)
        outbuf[rows, :] = (abuf[rows, :] + omg * b).astype(BF)
        pltpu.make_async_copy(outbuf.at[rows, :], out_hbm.at[rows, :], sem_out).start()
        return out_o[:M].astype(BF).astype(F32)

    with jax.named_scope("ph_pair"):
        jax.lax.fori_loop(0, N_PAIRS, pair, mem_ref[...].astype(F32))

    pltpu.make_async_copy(outbuf, out_hbm, sem_out).wait()


@functools.partial(jax.jit, static_argnames=("B_seg_len",))
def pallas_gated_mix__softmax_full_mha__memory_aug_recurrent_mem_tr__prompt_kernel(
    A_x: jax.Array,
    A_wqkv: jax.Array,
    A_wo: jax.Array,
    B_x: jax.Array,
    B_mem0: jax.Array,
    B_Wq: jax.Array,
    B_Wk: jax.Array,
    B_Wv: jax.Array,
    B_Wo: jax.Array,
    B_seg_len: int,
    gate_w: jax.Array,
):
    assert B_seg_len == SEG
    assert A_x.shape == (1, S, D)
    assert B_Wq.shape == (D, HB, DHB) and B_Wo.shape == (HB, DHB, D)

    any_spec = pl.BlockSpec(memory_space=pl.ANY)
    vmem_spec = pl.BlockSpec(memory_space=pltpu.VMEM)
    out = pl.pallas_call(
        _kernel,
        out_shape=jax.ShapeDtypeStruct((S, D), BF),
        in_specs=[any_spec, any_spec, any_spec, vmem_spec, any_spec, any_spec,
                  any_spec, any_spec, vmem_spec],
        out_specs=any_spec,
        scratch_shapes=[
            pltpu.VMEM((S, D), BF),
            pltpu.VMEM((3, D // 2, D), U32),
            pltpu.VMEM((D // 2, D), U32),
            pltpu.VMEM((S // 2, D), U32),
            pltpu.VMEM((D, S), BF),
            pltpu.VMEM((D // 2, S), U32),
            pltpu.VMEM((D, S), BF),
            pltpu.VMEM((S, D), F32),
            pltpu.VMEM((S, 128), F32),
            pltpu.VMEM((D // 2, HB * 384), U32),
            pltpu.VMEM((HB * DHB // 2, D), U32),
            pltpu.VMEM((N_HP * 3 + 1, D, 128), U32),
            pltpu.VMEM((S, D), BF),
            pltpu.VMEM((AHEAD, KB, QB), F32),
            pltpu.SMEM((1,), jnp.int32),
            pltpu.SemaphoreType.DMA((S // TB + 9,)),
            pltpu.SemaphoreType.DMA((N_HP,)),
            pltpu.SemaphoreType.DMA(()),
        ],
        compiler_params=pltpu.CompilerParams(vmem_limit_bytes=124 * 1024 * 1024),
    )(A_x.reshape(S, D), A_wqkv, A_wo, B_mem0.reshape(M, D),
      B_Wq, B_Wk, B_Wv, B_Wo.reshape(HB * DHB, D), gate_w)
    return out.reshape(1, S, D)
```

```python
import functools
import math

import jax
import jax.numpy as jnp
import jax.experimental.pallas as pl
import jax.experimental.pallas.tpu as pltpu

BF = jnp.bfloat16
F32 = jnp.float32
U32 = jnp.uint32

S = 2048
D = 1024
HA, DHA = 32, 32
HB, DHB = 32, 128
M = 8
SEG = 32
L = M + SEG

LOG2E = math.log2(math.e)
CA = DHA ** -0.5 * LOG2E
CB = DHB ** -0.5 * LOG2E
NEG_B = -1e9 * LOG2E

TB = 512
QB = 256
KB = 128
AHEAD = 4
UN = 16
GB = 4
NGB = HB // GB
NQ = S // QB
NK = S // KB
N_UNITS = HA * NQ
N_PAIRS = S // (2 * SEG)
N_HP = HB // 2


def _tree(op, xs):
    xs = list(xs)
    while len(xs) > 1:
        nxt = [op(xs[i], xs[i + 1]) for i in range(0, len(xs) - 1, 2)]
        if len(xs) % 2:
            nxt.append(xs[-1])
        xs = nxt
    return xs[0]


def _kernel(ax_hbm, wqkv_hbm, awo_hbm, mem_ref, bwq_hbm, bwk_hbm, bwv_hbm,
            bwo_hbm, gw_ref, out_hbm,
            ax, wqkv, awo, kbuf, qt, vt, ot, abuf, gbuf, wb, wob, stage, outbuf, scarry, spare_idx,
            sem_in, sem_st, sem_out):
    nblk = S // TB

    def ax_cp(i):
        r0 = pl.multiple_of(i * TB, TB)
        return pltpu.make_async_copy(ax_hbm.at[pl.ds(r0, TB), :], ax.at[pl.ds(r0, TB), :],
                                     sem_in.at[i])

    wqkv_u32 = wqkv_hbm.bitcast(U32)
    NC = 4
    CW = D // NC

    def wk_cp(c):
        c0 = pl.multiple_of(c * CW, CW)
        return pltpu.make_async_copy(wqkv_u32.at[:, pl.ds(D + c0, CW)],
                                     wqkv.at[1, :, pl.ds(c0, CW)], sem_in.at[nblk + 5 + c])

    def wqkv_cp(t):
        return pltpu.make_async_copy(wqkv_u32.at[:, pl.ds(t * D, D)], wqkv.at[t],
                                     sem_in.at[nblk + t])

    awo_cp = pltpu.make_async_copy(awo_hbm.bitcast(U32), awo, sem_in.at[nblk + 3])
    wob_cp = pltpu.make_async_copy(bwo_hbm.bitcast(U32), wob, sem_in.at[nblk + 4])

    bw_u32 = [r.bitcast(U32) for r in (bwq_hbm, bwk_hbm, bwv_hbm)]

    def stage_cp(hp, t, par):
        return pltpu.make_async_copy(bw_u32[t].at[:, par, hp, :],
                                     stage.at[(hp * 3 + t) * 2 + par], sem_st.at[hp])

    spare_idx[0] = N_HP * 6
    ax_cp(0).start()
    for c in range(NC):
        wk_cp(c).start()
    for i in range(1, nblk):
        ax_cp(i).start()
    wqkv_cp(0).start()
    wqkv_cp(2).start()

    ax_cp(0).wait()

    def k_proj0(c, carry):
        wk_cp(c).wait()
        c0 = pl.multiple_of(c * CW, CW)
        k = jnp.dot(ax[0:TB, :], pltpu.bitcast(wqkv[1, :, pl.ds(c0, CW)], BF),
                    preferred_element_type=F32)
        kbuf[0:TB // 2, pl.ds(c0, CW)] = pltpu.bitcast(k.astype(BF), U32)
        return carry

    def k_proj(i, c):
        ax_cp(i).wait()
        r0 = pl.multiple_of(i * TB, TB)
        rh = pl.multiple_of(i * (TB // 2), TB // 2)
        k = jnp.dot(ax[pl.ds(r0, TB), :], pltpu.bitcast(wqkv[1], BF), preferred_element_type=F32)
        kbuf[pl.ds(rh, TB // 2), :] = pltpu.bitcast(k.astype(BF), U32)
        return c

    with jax.named_scope("ph_kproj0"):
        jax.lax.fori_loop(0, NC, k_proj0, 0)
    with jax.named_scope("ph_kproj"):
        jax.lax.fori_loop(1, nblk, k_proj, 0)

    wqkv_cp(0).wait()
    wqkv_cp(2).wait()
    def start_stage(hp_lo, hp_hi):
        for hp in range(hp_lo, hp_hi):
            for t in range(3):
                for par in range(2):
                    stage_cp(hp, t, par).start(priority=1)

    start_stage(0, N_HP // 2)
    awo_cp.start(priority=1)
    wob_cp.start(priority=1)

    def qv_proj(i, c):
        r0 = pl.multiple_of(i * TB, TB)
        xb = ax[pl.ds(r0, TB), :]
        q = jnp.dot(xb, pltpu.bitcast(wqkv[0], BF), preferred_element_type=F32) * CA
        qt[:, pl.ds(r0, TB)] = q.T.astype(BF)
        v = jnp.dot(xb, pltpu.bitcast(wqkv[2], BF), preferred_element_type=F32)
        vt[:, pl.ds(r0, TB)] = pltpu.bitcast(v.T.astype(BF), U32)
        z = jnp.sum(xb.astype(F32) * gw_ref[...].astype(F32).reshape(1, D), axis=1, keepdims=True)
        gbuf[pl.ds(r0, TB), :] = jnp.broadcast_to(1.0 / (1.0 + jnp.exp(-z)), (TB, 128))
        return c

    with jax.named_scope("ph_qvproj"):
        jax.lax.fori_loop(0, nblk, qv_proj, 0)

    start_stage(N_HP // 2, N_HP)

    def unit_setup(u):
        h = u % HA
        g0 = pl.multiple_of((h // 4) * 128, 128)
        h0 = pl.multiple_of(h * DHA, DHA)
        q0 = pl.multiple_of((u // HA) * QB, QB)
        qg = pltpu.bitcast(qt[pl.ds(g0, 128), pl.ds(q0, QB)], U32)
        rows = jax.lax.broadcasted_iota(jnp.int32, (64, QB), 0)
        qm = pltpu.bitcast(jnp.where(rows // 16 == h % 4, qg, U32(0)), BF)
        return qm, g0, h0, q0

    def qk_chunk(setup, j):
        qm, g0, _, _ = setup
        kb = pltpu.bitcast(kbuf[j * KB // 2:(j + 1) * KB // 2, pl.ds(g0, 128)], BF)
        return jnp.dot(kb, qm, preferred_element_type=F32)

    def attn_iter(it, c):
        setup = [unit_setup(it * UN + k) for k in range(UN)]
        setup_next = unit_setup(jnp.minimum(it * UN + UN, N_UNITS - 1))
        items = [(uu, j) for uu in range(UN) for j in range(NK)]
        n = len(items)
        state = {}

        def pv(i, p, al, l):
            uu, j = items[i]
            _, _, h0, q0 = setup[uu]
            hh0 = pl.multiple_of(h0 // 2, DHA // 2)
            vtb = pltpu.bitcast(vt[pl.ds(hh0, DHA // 2), j * KB:(j + 1) * KB], BF)
            d = jnp.dot(vtb, p, preferred_element_type=F32)
            acc = d if j == 0 else state["acc"] * al + d
            state["acc"] = acc
            if j == NK - 1:
                o = acc / jnp.sum(l, axis=0, keepdims=True)
                ot[pl.ds(h0, DHA), pl.ds(q0, QB)] = o.astype(BF)

        ss = {i: scarry[i] for i in range(AHEAD)}
        m = l = None
        pend = None
        for i, (uu, j) in enumerate(items):
            if i + AHEAD < n:
                uu2, j2 = items[i + AHEAD]
                ss[i + AHEAD] = qk_chunk(setup[uu2], j2)
            else:
                scarry[i + AHEAD - n] = qk_chunk(setup_next, i + AHEAD - n)
            if pend is not None:
                pv(*pend)
            s = ss.pop(i)
            bm = _tree(jnp.maximum, [s[8 * r:8 * r + 8] for r in range(KB // 8)])
            bm = jnp.max(bm, axis=0, keepdims=True)
            if j == 0:
                m, al = bm, None
                p = jnp.exp2(s - m)
                l = _tree(jnp.add, [p[8 * r:8 * r + 8] for r in range(KB // 8)])
            else:
                mn = jnp.maximum(m, bm)
                al = jnp.exp2(m - mn)
                p = jnp.exp2(s - mn)
                l = l * al + _tree(jnp.add, [p[8 * r:8 * r + 8] for r in range(KB // 8)])
                m = mn
            pend = (i, p.astype(BF), al, l)
        pv(*pend)
        return c

    setup0 = unit_setup(0)
    for j in range(AHEAD):
        scarry[j] = qk_chunk(setup0, j)
    with jax.named_scope("ph_attn"):
        jax.lax.fori_loop(0, N_UNITS // UN, attn_iter, 0)

    awo_cp.wait()
    for hp in range(N_HP):
        pltpu.make_async_copy(stage.at[pl.ds(hp * 6, 6)], stage.at[pl.ds(hp * 6, 6)],
                              sem_st.at[hp]).wait()

    RS, CS, SUB = 4, 8, 32
    HP_IT = N_HP // nblk

    def relayout(hp, t, sub):
        nr = D // 2 // SUB
        ev = stage[(hp * 3 + t) * 2, sub * nr:(sub + 1) * nr, :]
        od = stage[(hp * 3 + t) * 2 + 1, sub * nr:(sub + 1) * nr, :]
        lo = (ev & U32(0xFFFF)) | (od << 16)
        hi = (ev >> 16) | (od & U32(0xFFFF0000))
        c0 = pl.multiple_of(hp * 768 + t * 128, 128)
        wb[sub * nr:(sub + 1) * nr, pl.ds(c0, 128)] = lo
        wb[sub * nr:(sub + 1) * nr, pl.ds(c0 + 384, 128)] = hi

    def a_out(i, c):
        r0 = pl.multiple_of(i * TB, TB)
        lhs = ot[:, pl.ds(r0, TB)].T
        pieces = [(i * HP_IT + k, t, sub) for k in range(HP_IT) for t in range(3)
                  for sub in range(SUB)]
        slots = [(cc, rr) for cc in range(CS) for rr in range(RS)]
        spare = spare_idx[0]
        rb, cw = TB // RS, D // CS
        for si, (cc, rr) in enumerate(slots):
            a = jnp.dot(lhs[rr * rb:(rr + 1) * rb], pltpu.bitcast(awo[:, cc * cw:(cc + 1) * cw], BF),
                        preferred_element_type=F32)
            rows = pl.ds(pl.multiple_of(r0 + rr * rb, rb), rb)
            abuf[rows, cc * cw:(cc + 1) * cw] = a * gbuf[rows, :]
            stage[spare, 0:8, :] = pltpu.bitcast(a[0:8, 0:128], U32)
            for q, p in enumerate(pieces):
                if q * len(slots) // len(pieces) == si:
                    relayout(*p)
        return c

    with jax.named_scope("ph_aout"):
        jax.lax.fori_loop(0, nblk, a_out, 0)

    wob_cp.wait()

    NE, NO = 32, 48
    ri = jax.lax.broadcasted_iota(jnp.int32, (NE, L), 0)
    ci = jax.lax.broadcasted_iota(jnp.int32, (NE, L), 1)
    mask_e = (ri < M) | (ri >= ci)
    fill_e = NEG_B
    ri = jax.lax.broadcasted_iota(jnp.int32, (NO, 2 * L), 0)
    ci = jax.lax.broadcasted_iota(jnp.int32, (NO, 2 * L), 1)
    own = ((ri < L) & (ci >= L)) | ((ri >= L) & (ci < L))
    qi = jnp.where(ri < L, ri, ri - 8)
    ki = jnp.where(ci < L, ci, ci - L)
    mask_o = own & ((qi < M) | (qi >= ki))
    fill_o = jnp.where(own, NEG_B, -3e38)

    def qkv_dot(lhs, g):
        w = pltpu.bitcast(wb[:, g * GB * 384:(g + 1) * GB * 384], BF)
        return jnp.dot(lhs, w, preferred_element_type=F32)

    def qk_dots(qrows, kvrows):
        res = []
        for hh in range(GB):
            b = hh * 384
            q = (qrows[:, b:b + 128] * CB).astype(BF)
            k = kvrows[:, b + 128:b + 256].astype(BF)
            v = kvrows[:, b + 256:b + 384].astype(BF)
            s = jax.lax.dot_general(q, k, (((1,), (1,)), ((), ())), preferred_element_type=F32)
            res.append((s, v))
        return res

    def pv_dots(sv, mask, fill):
        outs = []
        for s, v in sv:
            s = jnp.where(mask, s, fill)
            mx = jnp.max(s, axis=1, keepdims=True)
            p = jnp.exp2(s - mx)
            l = jnp.sum(p, axis=1, keepdims=True)
            o = jnp.dot(p.astype(BF), v, preferred_element_type=F32)
            outs.append(o / l)
        return jnp.concatenate(outs, axis=1)

    def wo_dot(lhs, g):
        w = pltpu.bitcast(wob[g * GB * 64:(g + 1) * GB * 64, :], BF)
        return jnp.dot(lhs.astype(BF), w, preferred_element_type=F32)

    def run_step(lhs, rows_fn, mask, fill):
        qkv, sv, o = {}, {}, {}
        out = None
        qkv[0] = qkv_dot(lhs, 0)
        for g in range(NGB + 2):
            if g + 1 < NGB:
                qkv[g + 1] = qkv_dot(lhs, g + 1)
            if 0 <= g - 1 < NGB:
                o[g - 1] = pv_dots(sv[g - 1], mask, fill)
            if g < NGB:
                sv[g] = qk_dots(*rows_fn(qkv[g], g))
            if 0 <= g - 2 < NGB:
                d = wo_dot(o[g - 2], g - 2)
                out = d if out is None else out + d
        return out, qkv

    def pair(j, mem):
        t0 = pl.multiple_of(j * 2 * SEG, 2 * SEG)
        t1 = pl.multiple_of(j * 2 * SEG + SEG, SEG)
        x_e = ax[pl.ds(t0, 48), :].astype(F32)[:40]
        x_o = ax[pl.ds(t1, SEG), :].astype(F32)[8:]
        lhs_e = jnp.concatenate([mem, x_e], axis=0).astype(BF)
        out_e, qkv_e = run_step(lhs_e, lambda q, g: (q[:NE], q[:L]), mask_e, fill_e)
        mem1 = out_e[:M].astype(BF).astype(F32)
        lhs_o = jnp.concatenate([mem1, x_o], axis=0).astype(BF)

        def rows_o(q, g):
            e = qkv_e[g]
            seg_o = [q[:8], e[40:48], q[8:32]]
            return (jnp.concatenate(seg_o + [e[32:40]], axis=0),
                    jnp.concatenate([e[:L]] + seg_o, axis=0))

        out_o, _ = run_step(lhs_o, rows_o, mask_o, fill_o)
        b = jnp.concatenate([out_e[8:32], out_o[40:48], out_o[8:40]], axis=0)
        rows = pl.ds(t0, 2 * SEG)
        omg = jnp.concatenate([1.0 - gbuf[rows, :]] * (D // 128), axis=1)
        outbuf[rows, :] = (abuf[rows, :] + omg * b).astype(BF)
        pltpu.make_async_copy(outbuf.at[rows, :], out_hbm.at[rows, :], sem_out).start()
        return out_o[:M].astype(BF).astype(F32)

    with jax.named_scope("ph_pair"):
        jax.lax.fori_loop(0, N_PAIRS, pair, mem_ref[...].astype(F32))

    pltpu.make_async_copy(outbuf, out_hbm, sem_out).wait()


@functools.partial(jax.jit, static_argnames=("B_seg_len",))
def pallas_gated_mix__softmax_full_mha__memory_aug_recurrent_mem_tr__prompt_kernel(
    A_x: jax.Array,
    A_wqkv: jax.Array,
    A_wo: jax.Array,
    B_x: jax.Array,
    B_mem0: jax.Array,
    B_Wq: jax.Array,
    B_Wk: jax.Array,
    B_Wv: jax.Array,
    B_Wo: jax.Array,
    B_seg_len: int,
    gate_w: jax.Array,
):
    assert B_seg_len == SEG
    assert A_x.shape == (1, S, D)
    assert B_Wq.shape == (D, HB, DHB) and B_Wo.shape == (HB, DHB, D)

    any_spec = pl.BlockSpec(memory_space=pl.ANY)
    vmem_spec = pl.BlockSpec(memory_space=pltpu.VMEM)
    out = pl.pallas_call(
        _kernel,
        out_shape=jax.ShapeDtypeStruct((S, D), BF),
        in_specs=[any_spec, any_spec, any_spec, vmem_spec, any_spec, any_spec,
                  any_spec, any_spec, vmem_spec],
        out_specs=any_spec,
        scratch_shapes=[
            pltpu.VMEM((S, D), BF),
            pltpu.VMEM((3, D // 2, D), U32),
            pltpu.VMEM((D // 2, D), U32),
            pltpu.VMEM((S // 2, D), U32),
            pltpu.VMEM((D, S), BF),
            pltpu.VMEM((D // 2, S), U32),
            pltpu.VMEM((D, S), BF),
            pltpu.VMEM((S, D), F32),
            pltpu.VMEM((S, 128), F32),
            pltpu.VMEM((D // 2, HB * 384), U32),
            pltpu.VMEM((HB * DHB // 2, D), U32),
            pltpu.VMEM((N_HP * 6 + 1, D // 2, 128), U32),
            pltpu.VMEM((S, D), BF),
            pltpu.VMEM((AHEAD, KB, QB), F32),
            pltpu.SMEM((1,), jnp.int32),
            pltpu.SemaphoreType.DMA((S // TB + 9,)),
            pltpu.SemaphoreType.DMA((N_HP,)),
            pltpu.SemaphoreType.DMA(()),
        ],
        compiler_params=pltpu.CompilerParams(vmem_limit_bytes=124 * 1024 * 1024),
    )(A_x.reshape(S, D), A_wqkv, A_wo, B_mem0.reshape(M, D),
      *[w.reshape(D // 2, 2, HB, DHB) for w in (B_Wq, B_Wk, B_Wv)],
      B_Wo.reshape(HB * DHB, D), gate_w)
    return out.reshape(1, S, D)
```

```python
import functools
import math

import jax
import jax.numpy as jnp
import jax.experimental.pallas as pl
import jax.experimental.pallas.tpu as pltpu

BF = jnp.bfloat16
F32 = jnp.float32
U32 = jnp.uint32

S = 2048
D = 1024
HA, DHA = 32, 32
HB, DHB = 32, 128
M = 8
SEG = 32
L = M + SEG

LOG2E = math.log2(math.e)
CA = DHA ** -0.5 * LOG2E
CB = DHB ** -0.5 * LOG2E
NEG_B = -1e9 * LOG2E

TB = 512
QB = 256
KB = 128
AHEAD = 4
UN = 16
GB = 2
NGB = HB // GB
PV_LAG, WO_LAG = 2, 3
NQ = S // QB
NK = S // KB
N_UNITS = HA * NQ
N_PAIRS = S // (2 * SEG)
N_HP = HB // 2


def _tree(op, xs):
    xs = list(xs)
    while len(xs) > 1:
        nxt = [op(xs[i], xs[i + 1]) for i in range(0, len(xs) - 1, 2)]
        if len(xs) % 2:
            nxt.append(xs[-1])
        xs = nxt
    return xs[0]


def _kernel(ax_hbm, wqkv_hbm, awo_hbm, mem_ref, bwq_hbm, bwk_hbm, bwv_hbm,
            bwo_hbm, gw_ref, out_hbm,
            ax, wqkv, awo, kbuf, qt, vt, ot, abuf, gbuf, wb, wob, stage, outbuf, scarry, spare_idx,
            sem_in, sem_st, sem_out):
    nblk = S // TB

    def ax_cp(i):
        r0 = pl.multiple_of(i * TB, TB)
        return pltpu.make_async_copy(ax_hbm.at[pl.ds(r0, TB), :], ax.at[pl.ds(r0, TB), :],
                                     sem_in.at[i])

    wqkv_u32 = wqkv_hbm.bitcast(U32)
    NC = 4
    CW = D // NC

    def wk_cp(c):
        c0 = pl.multiple_of(c * CW, CW)
        return pltpu.make_async_copy(wqkv_u32.at[:, pl.ds(D + c0, CW)],
                                     wqkv.at[1, :, pl.ds(c0, CW)], sem_in.at[nblk + 5 + c])

    def wqkv_cp(t):
        return pltpu.make_async_copy(wqkv_u32.at[:, pl.ds(t * D, D)], wqkv.at[t],
                                     sem_in.at[nblk + t])

    awo_cp = pltpu.make_async_copy(awo_hbm.bitcast(U32), awo, sem_in.at[nblk + 3])
    wob_cp = pltpu.make_async_copy(bwo_hbm.bitcast(U32), wob, sem_in.at[nblk + 4])

    bw_u32 = [r.bitcast(U32) for r in (bwq_hbm, bwk_hbm, bwv_hbm)]

    def stage_cp(hp, t, par):
        return pltpu.make_async_copy(bw_u32[t].at[:, par, hp, :],
                                     stage.at[(hp * 3 + t) * 2 + par], sem_st.at[hp])

    spare_idx[0] = N_HP * 6
    ax_cp(0).start()
    for c in range(NC):
        wk_cp(c).start()
    for i in range(1, nblk):
        ax_cp(i).start()
    wqkv_cp(0).start()
    wqkv_cp(2).start()

    ax_cp(0).wait()

    def k_proj0(c, carry):
        wk_cp(c).wait()
        c0 = pl.multiple_of(c * CW, CW)
        k = jnp.dot(ax[0:TB, :], pltpu.bitcast(wqkv[1, :, pl.ds(c0, CW)], BF),
                    preferred_element_type=F32)
        kbuf[0:TB // 2, pl.ds(c0, CW)] = pltpu.bitcast(k.astype(BF), U32)
        return carry

    def k_proj(i, c):
        ax_cp(i).wait()
        r0 = pl.multiple_of(i * TB, TB)
        rh = pl.multiple_of(i * (TB // 2), TB // 2)
        k = jnp.dot(ax[pl.ds(r0, TB), :], pltpu.bitcast(wqkv[1], BF), preferred_element_type=F32)
        kbuf[pl.ds(rh, TB // 2), :] = pltpu.bitcast(k.astype(BF), U32)
        return c

    with jax.named_scope("ph_kproj0"):
        jax.lax.fori_loop(0, NC, k_proj0, 0)
    with jax.named_scope("ph_kproj"):
        jax.lax.fori_loop(1, nblk, k_proj, 0)

    wqkv_cp(0).wait()
    wqkv_cp(2).wait()
    def start_stage(hp_lo, hp_hi):
        for hp in range(hp_lo, hp_hi):
            for t in range(3):
                for par in range(2):
                    stage_cp(hp, t, par).start(priority=1)

    start_stage(0, N_HP // 2)
    awo_cp.start(priority=1)
    wob_cp.start(priority=1)

    def qv_proj(i, c):
        r0 = pl.multiple_of(i * TB, TB)
        xb = ax[pl.ds(r0, TB), :]
        q = jnp.dot(xb, pltpu.bitcast(wqkv[0], BF), preferred_element_type=F32) * CA
        qt[:, pl.ds(r0, TB)] = q.T.astype(BF)
        v = jnp.dot(xb, pltpu.bitcast(wqkv[2], BF), preferred_element_type=F32)
        vt[:, pl.ds(r0, TB)] = pltpu.bitcast(v.T.astype(BF), U32)
        z = jnp.sum(xb.astype(F32) * gw_ref[...].astype(F32).reshape(1, D), axis=1, keepdims=True)
        gbuf[pl.ds(r0, TB), :] = jnp.broadcast_to(1.0 / (1.0 + jnp.exp(-z)), (TB, 128))
        return c

    with jax.named_scope("ph_qvproj"):
        jax.lax.fori_loop(0, nblk, qv_proj, 0)

    start_stage(N_HP // 2, N_HP)

    def unit_setup(u):
        h = u % HA
        g0 = pl.multiple_of((h // 4) * 128, 128)
        h0 = pl.multiple_of(h * DHA, DHA)
        q0 = pl.multiple_of((u // HA) * QB, QB)
        qg = pltpu.bitcast(qt[pl.ds(g0, 128), pl.ds(q0, QB)], U32)
        rows = jax.lax.broadcasted_iota(jnp.int32, (64, QB), 0)
        qm = pltpu.bitcast(jnp.where(rows // 16 == h % 4, qg, U32(0)), BF)
        return qm, g0, h0, q0

    def qk_chunk(setup, j):
        qm, g0, _, _ = setup
        kb = pltpu.bitcast(kbuf[j * KB // 2:(j + 1) * KB // 2, pl.ds(g0, 128)], BF)
        return jnp.dot(kb, qm, preferred_element_type=F32)

    def attn_iter(it, c):
        setup = [unit_setup(it * UN + k) for k in range(UN)]
        setup_next = unit_setup(jnp.minimum(it * UN + UN, N_UNITS - 1))
        items = [(uu, j) for uu in range(UN) for j in range(NK)]
        n = len(items)
        state = {}

        def pv(i, p, al, l):
            uu, j = items[i]
            _, _, h0, q0 = setup[uu]
            hh0 = pl.multiple_of(h0 // 2, DHA // 2)
            vtb = pltpu.bitcast(vt[pl.ds(hh0, DHA // 2), j * KB:(j + 1) * KB], BF)
            d = jnp.dot(vtb, p, preferred_element_type=F32)
            acc = d if j == 0 else state["acc"] * al + d
            state["acc"] = acc
            if j == NK - 1:
                o = acc / jnp.sum(l, axis=0, keepdims=True)
                ot[pl.ds(h0, DHA), pl.ds(q0, QB)] = o.astype(BF)

        ss = {i: scarry[i] for i in range(AHEAD)}
        m = l = None
        pend = None
        for i, (uu, j) in enumerate(items):
            if i + AHEAD < n:
                uu2, j2 = items[i + AHEAD]
                ss[i + AHEAD] = qk_chunk(setup[uu2], j2)
            else:
                scarry[i + AHEAD - n] = qk_chunk(setup_next, i + AHEAD - n)
            if pend is not None:
                pv(*pend)
            s = ss.pop(i)
            bm = _tree(jnp.maximum, [s[8 * r:8 * r + 8] for r in range(KB // 8)])
            bm = jnp.max(bm, axis=0, keepdims=True)
            if j == 0:
                m, al = bm, None
                p = jnp.exp2(s - m)
                l = _tree(jnp.add, [p[8 * r:8 * r + 8] for r in range(KB // 8)])
            else:
                mn = jnp.maximum(m, bm)
                al = jnp.exp2(m - mn)
                p = jnp.exp2(s - mn)
                l = l * al + _tree(jnp.add, [p[8 * r:8 * r + 8] for r in range(KB // 8)])
                m = mn
            pend = (i, p.astype(BF), al, l)
        pv(*pend)
        return c

    setup0 = unit_setup(0)
    for j in range(AHEAD):
        scarry[j] = qk_chunk(setup0, j)
    with jax.named_scope("ph_attn"):
        jax.lax.fori_loop(0, N_UNITS // UN, attn_iter, 0)

    awo_cp.wait()
    for hp in range(N_HP):
        pltpu.make_async_copy(stage.at[pl.ds(hp * 6, 6)], stage.at[pl.ds(hp * 6, 6)],
                              sem_st.at[hp]).wait()

    RS, CS, SUB = 4, 8, 32
    HP_IT = N_HP // nblk

    def relayout(hp, t, sub):
        nr = D // 2 // SUB
        ev = stage[(hp * 3 + t) * 2, sub * nr:(sub + 1) * nr, :]
        od = stage[(hp * 3 + t) * 2 + 1, sub * nr:(sub + 1) * nr, :]
        lo = (ev & U32(0xFFFF)) | (od << 16)
        hi = (ev >> 16) | (od & U32(0xFFFF0000))
        c0 = pl.multiple_of(hp * 768 + t * 128, 128)
        wb[sub * nr:(sub + 1) * nr, pl.ds(c0, 128)] = lo
        wb[sub * nr:(sub + 1) * nr, pl.ds(c0 + 384, 128)] = hi

    def a_out(i, c):
        r0 = pl.multiple_of(i * TB, TB)
        lhs = ot[:, pl.ds(r0, TB)].T
        pieces = [(i * HP_IT + k, t, sub) for k in range(HP_IT) for t in range(3)
                  for sub in range(SUB)]
        slots = [(cc, rr) for cc in range(CS) for rr in range(RS)]
        spare = spare_idx[0]
        rb, cw = TB // RS, D // CS
        for si, (cc, rr) in enumerate(slots):
            a = jnp.dot(lhs[rr * rb:(rr + 1) * rb], pltpu.bitcast(awo[:, cc * cw:(cc + 1) * cw], BF),
                        preferred_element_type=F32)
            rows = pl.ds(pl.multiple_of(r0 + rr * rb, rb), rb)
            abuf[rows, cc * cw:(cc + 1) * cw] = a * gbuf[rows, :]
            stage[spare, 0:8, :] = pltpu.bitcast(a[0:8, 0:128], U32)
            for q, p in enumerate(pieces):
                if q * len(slots) // len(pieces) == si:
                    relayout(*p)
        return c

    with jax.named_scope("ph_aout"):
        jax.lax.fori_loop(0, nblk, a_out, 0)

    wob_cp.wait()

    NE, NO = 32, 48
    ri = jax.lax.broadcasted_iota(jnp.int32, (NE, L), 0)
    ci = jax.lax.broadcasted_iota(jnp.int32, (NE, L), 1)
    mask_e = (ri < M) | (ri >= ci)
    fill_e = NEG_B
    ri = jax.lax.broadcasted_iota(jnp.int32, (NO, 2 * L), 0)
    ci = jax.lax.broadcasted_iota(jnp.int32, (NO, 2 * L), 1)
    own = ((ri < L) & (ci >= L)) | ((ri >= L) & (ci < L))
    qi = jnp.where(ri < L, ri, ri - 8)
    ki = jnp.where(ci < L, ci, ci - L)
    mask_o = own & ((qi < M) | (qi >= ki))
    fill_o = jnp.where(own, NEG_B, -3e38)

    def qkv_dot(lhs, g):
        w = pltpu.bitcast(wb[:, g * GB * 384:(g + 1) * GB * 384], BF)
        return jnp.dot(lhs, w, preferred_element_type=F32)

    def qk_dots(qrows, kvrows):
        res = []
        for hh in range(GB):
            b = hh * 384
            q = (qrows[:, b:b + 128] * CB).astype(BF)
            k = kvrows[:, b + 128:b + 256].astype(BF)
            v = kvrows[:, b + 256:b + 384].astype(BF)
            s = jax.lax.dot_general(q, k, (((1,), (1,)), ((), ())), preferred_element_type=F32)
            res.append((s, v))
        return res

    def pv_dots(sv, mask, fill):
        outs = []
        for s, v in sv:
            s = jnp.where(mask, s, fill)
            mx = jnp.max(s, axis=1, keepdims=True)
            p = jnp.exp2(s - mx)
            l = jnp.sum(p, axis=1, keepdims=True)
            o = jnp.dot(p.astype(BF), v, preferred_element_type=F32)
            outs.append(o / l)
        return jnp.concatenate(outs, axis=1)

    def wo_dot(lhs, g):
        w = pltpu.bitcast(wob[g * GB * 64:(g + 1) * GB * 64, :], BF)
        return jnp.dot(lhs.astype(BF), w, preferred_element_type=F32)

    def run_step(lhs, rows_fn, mask, fill):
        qkv, sv, o = {}, {}, {}
        out = None
        qkv[0] = qkv_dot(lhs, 0)
        for g in range(NGB + WO_LAG):
            if g + 1 < NGB:
                qkv[g + 1] = qkv_dot(lhs, g + 1)
            if g < NGB:
                sv[g] = qk_dots(*rows_fn(qkv[g], g))
            if 0 <= g - PV_LAG < NGB:
                o[g - PV_LAG] = pv_dots(sv[g - PV_LAG], mask, fill)
            if 0 <= g - WO_LAG < NGB:
                d = wo_dot(o[g - WO_LAG], g - WO_LAG)
                out = d if out is None else out + d
        return out, qkv

    def pair(j, mem):
        t0 = pl.multiple_of(j * 2 * SEG, 2 * SEG)
        t1 = pl.multiple_of(j * 2 * SEG + SEG, SEG)
        x_e = ax[pl.ds(t0, 48), :].astype(F32)[:40]
        x_o = ax[pl.ds(t1, SEG), :].astype(F32)[8:]
        lhs_e = jnp.concatenate([mem, x_e], axis=0).astype(BF)
        out_e, qkv_e = run_step(lhs_e, lambda q, g: (q[:NE], q[:L]), mask_e, fill_e)
        mem1 = out_e[:M].astype(BF).astype(F32)
        lhs_o = jnp.concatenate([mem1, x_o], axis=0).astype(BF)

        def rows_o(q, g):
            e = qkv_e[g]
            seg_o = [q[:8], e[40:48], q[8:32]]
            return (jnp.concatenate(seg_o + [e[32:40]], axis=0),
                    jnp.concatenate([e[:L]] + seg_o, axis=0))

        out_o, _ = run_step(lhs_o, rows_o, mask_o, fill_o)
        b = jnp.concatenate([out_e[8:32], out_o[40:48], out_o[8:40]], axis=0)
        rows = pl.ds(t0, 2 * SEG)
        omg = jnp.concatenate([1.0 - gbuf[rows, :]] * (D // 128), axis=1)
        outbuf[rows, :] = (abuf[rows, :] + omg * b).astype(BF)
        pltpu.make_async_copy(outbuf.at[rows, :], out_hbm.at[rows, :], sem_out).start()
        return out_o[:M].astype(BF).astype(F32)

    with jax.named_scope("ph_pair"):
        jax.lax.fori_loop(0, N_PAIRS, pair, mem_ref[...].astype(F32))

    pltpu.make_async_copy(outbuf, out_hbm, sem_out).wait()


@functools.partial(jax.jit, static_argnames=("B_seg_len",))
def pallas_gated_mix__softmax_full_mha__memory_aug_recurrent_mem_tr__prompt_kernel(
    A_x: jax.Array,
    A_wqkv: jax.Array,
    A_wo: jax.Array,
    B_x: jax.Array,
    B_mem0: jax.Array,
    B_Wq: jax.Array,
    B_Wk: jax.Array,
    B_Wv: jax.Array,
    B_Wo: jax.Array,
    B_seg_len: int,
    gate_w: jax.Array,
):
    assert B_seg_len == SEG
    assert A_x.shape == (1, S, D)
    assert B_Wq.shape == (D, HB, DHB) and B_Wo.shape == (HB, DHB, D)

    any_spec = pl.BlockSpec(memory_space=pl.ANY)
    vmem_spec = pl.BlockSpec(memory_space=pltpu.VMEM)
    out = pl.pallas_call(
        _kernel,
        out_shape=jax.ShapeDtypeStruct((S, D), BF),
        in_specs=[any_spec, any_spec, any_spec, vmem_spec, any_spec, any_spec,
                  any_spec, any_spec, vmem_spec],
        out_specs=any_spec,
        scratch_shapes=[
            pltpu.VMEM((S, D), BF),
            pltpu.VMEM((3, D // 2, D), U32),
            pltpu.VMEM((D // 2, D), U32),
            pltpu.VMEM((S // 2, D), U32),
            pltpu.VMEM((D, S), BF),
            pltpu.VMEM((D // 2, S), U32),
            pltpu.VMEM((D, S), BF),
            pltpu.VMEM((S, D), F32),
            pltpu.VMEM((S, 128), F32),
            pltpu.VMEM((D // 2, HB * 384), U32),
            pltpu.VMEM((HB * DHB // 2, D), U32),
            pltpu.VMEM((N_HP * 6 + 1, D // 2, 128), U32),
            pltpu.VMEM((S, D), BF),
            pltpu.VMEM((AHEAD, KB, QB), F32),
            pltpu.SMEM((1,), jnp.int32),
            pltpu.SemaphoreType.DMA((S // TB + 9,)),
            pltpu.SemaphoreType.DMA((N_HP,)),
            pltpu.SemaphoreType.DMA(()),
        ],
        compiler_params=pltpu.CompilerParams(vmem_limit_bytes=124 * 1024 * 1024),
    )(A_x.reshape(S, D), A_wqkv, A_wo, B_mem0.reshape(M, D),
      *[w.reshape(D // 2, 2, HB, DHB) for w in (B_Wq, B_Wk, B_Wv)],
      B_Wo.reshape(HB * DHB, D), gate_w)
    return out.reshape(1, S, D)
```

```python
import functools
import math

import jax
import jax.numpy as jnp
import jax.experimental.pallas as pl
import jax.experimental.pallas.tpu as pltpu

BF = jnp.bfloat16
F32 = jnp.float32
U32 = jnp.uint32

S = 2048
D = 1024
HA, DHA = 32, 32
HB, DHB = 32, 128
M = 8
SEG = 32
L = M + SEG

LOG2E = math.log2(math.e)
CA = DHA ** -0.5 * LOG2E
CB = DHB ** -0.5 * LOG2E
NEG_B = -1e9 * LOG2E

TB = 512
QB = 256
KB = 128
AHEAD = 4
UN = 16
GB = 2
NGB = HB // GB
PV_LAG, WO_LAG = 2, 3
NQ = S // QB
NK = S // KB
N_UNITS = HA * NQ
N_PAIRS = S // (2 * SEG)
N_HP = HB // 2


def _tree(op, xs):
    xs = list(xs)
    while len(xs) > 1:
        nxt = [op(xs[i], xs[i + 1]) for i in range(0, len(xs) - 1, 2)]
        if len(xs) % 2:
            nxt.append(xs[-1])
        xs = nxt
    return xs[0]


def _kernel(ax_hbm, wqkv_hbm, awo_hbm, mem_ref, bwq_hbm, bwk_hbm, bwv_hbm,
            bwo_hbm, gw_ref, out_hbm,
            ax, wqkv, awo, kbuf, qt, vt, ot, abuf, gbuf, wb, wob, stage, outbuf, scarry, spare_idx,
            sem_in, sem_st, sem_out):
    nblk = S // TB

    def ax_cp(i):
        r0 = pl.multiple_of(i * TB, TB)
        return pltpu.make_async_copy(ax_hbm.at[pl.ds(r0, TB), :], ax.at[pl.ds(r0, TB), :],
                                     sem_in.at[i])

    wqkv_u32 = wqkv_hbm.bitcast(U32)
    NC = 4
    CW = D // NC

    def wk_cp(c):
        c0 = pl.multiple_of(c * CW, CW)
        return pltpu.make_async_copy(wqkv_u32.at[:, pl.ds(D + c0, CW)],
                                     wqkv.at[1, :, pl.ds(c0, CW)], sem_in.at[nblk + 5 + c])

    def wqkv_cp(t):
        return pltpu.make_async_copy(wqkv_u32.at[:, pl.ds(t * D, D)], wqkv.at[t],
                                     sem_in.at[nblk + t])

    awo_cp = pltpu.make_async_copy(awo_hbm.bitcast(U32), awo, sem_in.at[nblk + 3])
    wob_cp = pltpu.make_async_copy(bwo_hbm.bitcast(U32), wob, sem_in.at[nblk + 4])

    bw_u32 = [r.bitcast(U32) for r in (bwq_hbm, bwk_hbm, bwv_hbm)]

    def stage_cp(hp, t, par):
        return pltpu.make_async_copy(bw_u32[t].at[:, par, hp, :],
                                     stage.at[(hp * 3 + t) * 2 + par], sem_st.at[hp])

    spare_idx[0] = N_HP * 6
    ax_cp(0).start()
    for c in range(NC):
        wk_cp(c).start()
    for i in range(1, nblk):
        ax_cp(i).start()
    wqkv_cp(0).start()
    wqkv_cp(2).start()

    ax_cp(0).wait()

    def k_proj0(c, carry):
        wk_cp(c).wait()
        c0 = pl.multiple_of(c * CW, CW)
        k = jnp.dot(ax[0:TB, :], pltpu.bitcast(wqkv[1, :, pl.ds(c0, CW)], BF),
                    preferred_element_type=F32)
        kbuf[0:TB // 2, pl.ds(c0, CW)] = pltpu.bitcast(k.astype(BF), U32)
        return carry

    def k_proj(i, c):
        ax_cp(i).wait()
        r0 = pl.multiple_of(i * TB, TB)
        rh = pl.multiple_of(i * (TB // 2), TB // 2)
        k = jnp.dot(ax[pl.ds(r0, TB), :], pltpu.bitcast(wqkv[1], BF), preferred_element_type=F32)
        kbuf[pl.ds(rh, TB // 2), :] = pltpu.bitcast(k.astype(BF), U32)
        return c

    with jax.named_scope("ph_kproj0"):
        jax.lax.fori_loop(0, NC, k_proj0, 0)
    with jax.named_scope("ph_kproj"):
        jax.lax.fori_loop(1, nblk, k_proj, 0)

    wqkv_cp(0).wait()
    wqkv_cp(2).wait()
    def start_stage(hp_lo, hp_hi):
        for hp in range(hp_lo, hp_hi):
            for t in range(3):
                for par in range(2):
                    stage_cp(hp, t, par).start(priority=1)

    start_stage(0, N_HP // 4)
    awo_cp.start(priority=1)
    wob_cp.start(priority=1)

    def qv_proj(i, c):
        r0 = pl.multiple_of(i * TB, TB)
        xb = ax[pl.ds(r0, TB), :]
        q = jnp.dot(xb, pltpu.bitcast(wqkv[0], BF), preferred_element_type=F32) * CA
        qt[:, pl.ds(r0, TB)] = q.T.astype(BF)
        v = jnp.dot(xb, pltpu.bitcast(wqkv[2], BF), preferred_element_type=F32)
        vt[:, pl.ds(r0, TB)] = pltpu.bitcast(v.T.astype(BF), U32)
        z = jnp.sum(xb.astype(F32) * gw_ref[...].astype(F32).reshape(1, D), axis=1, keepdims=True)
        gbuf[pl.ds(r0, TB), :] = jnp.broadcast_to(1.0 / (1.0 + jnp.exp(-z)), (TB, 128))
        return c

    with jax.named_scope("ph_qvproj"):
        jax.lax.fori_loop(0, nblk, qv_proj, 0)

    start_stage(N_HP // 4, 3 * N_HP // 4)

    def unit_setup(u):
        h = u % HA
        g0 = pl.multiple_of((h // 4) * 128, 128)
        h0 = pl.multiple_of(h * DHA, DHA)
        q0 = pl.multiple_of((u // HA) * QB, QB)
        qg = pltpu.bitcast(qt[pl.ds(g0, 128), pl.ds(q0, QB)], U32)
        rows = jax.lax.broadcasted_iota(jnp.int32, (64, QB), 0)
        qm = pltpu.bitcast(jnp.where(rows // 16 == h % 4, qg, U32(0)), BF)
        return qm, g0, h0, q0

    def qk_chunk(setup, j):
        qm, g0, _, _ = setup
        kb = pltpu.bitcast(kbuf[j * KB // 2:(j + 1) * KB // 2, pl.ds(g0, 128)], BF)
        return jnp.dot(kb, qm, preferred_element_type=F32)

    def attn_iter(it, c):
        @pl.when(it == 4)
        def _():
            start_stage(3 * N_HP // 4, N_HP)

        setup = [unit_setup(it * UN + k) for k in range(UN)]
        setup_next = unit_setup(jnp.minimum(it * UN + UN, N_UNITS - 1))
        items = [(uu, j) for uu in range(UN) for j in range(NK)]
        n = len(items)
        state = {}

        def pv(i, p, al, l):
            uu, j = items[i]
            _, _, h0, q0 = setup[uu]
            hh0 = pl.multiple_of(h0 // 2, DHA // 2)
            vtb = pltpu.bitcast(vt[pl.ds(hh0, DHA // 2), j * KB:(j + 1) * KB], BF)
            d = jnp.dot(vtb, p, preferred_element_type=F32)
            acc = d if j == 0 else state["acc"] * al + d
            state["acc"] = acc
            if j == NK - 1:
                o = acc / jnp.sum(l, axis=0, keepdims=True)
                ot[pl.ds(h0, DHA), pl.ds(q0, QB)] = o.astype(BF)

        ss = {i: scarry[i] for i in range(AHEAD)}
        m = l = None
        pend = None
        for i, (uu, j) in enumerate(items):
            if i + AHEAD < n:
                uu2, j2 = items[i + AHEAD]
                ss[i + AHEAD] = qk_chunk(setup[uu2], j2)
            else:
                scarry[i + AHEAD - n] = qk_chunk(setup_next, i + AHEAD - n)
            if pend is not None:
                pv(*pend)
            s = ss.pop(i)
            bm = _tree(jnp.maximum, [s[8 * r:8 * r + 8] for r in range(KB // 8)])
            bm = jnp.max(bm, axis=0, keepdims=True)
            if j == 0:
                m, al = bm, None
                p = jnp.exp2(s - m)
                l = _tree(jnp.add, [p[8 * r:8 * r + 8] for r in range(KB // 8)])
            else:
                mn = jnp.maximum(m, bm)
                al = jnp.exp2(m - mn)
                p = jnp.exp2(s - mn)
                l = l * al + _tree(jnp.add, [p[8 * r:8 * r + 8] for r in range(KB // 8)])
                m = mn
            pend = (i, p.astype(BF), al, l)
        pv(*pend)
        return c

    setup0 = unit_setup(0)
    for j in range(AHEAD):
        scarry[j] = qk_chunk(setup0, j)
    with jax.named_scope("ph_attn"):
        jax.lax.fori_loop(0, N_UNITS // UN, attn_iter, 0)

    awo_cp.wait()
    for hp in range(N_HP):
        pltpu.make_async_copy(stage.at[pl.ds(hp * 6, 6)], stage.at[pl.ds(hp * 6, 6)],
                              sem_st.at[hp]).wait()

    RS, CS, SUB = 4, 8, 32
    HP_IT = N_HP // nblk

    def relayout(hp, t, sub):
        nr = D // 2 // SUB
        ev = stage[(hp * 3 + t) * 2, sub * nr:(sub + 1) * nr, :]
        od = stage[(hp * 3 + t) * 2 + 1, sub * nr:(sub + 1) * nr, :]
        lo = (ev & U32(0xFFFF)) | (od << 16)
        hi = (ev >> 16) | (od & U32(0xFFFF0000))
        c0 = pl.multiple_of(hp * 768 + t * 128, 128)
        wb[sub * nr:(sub + 1) * nr, pl.ds(c0, 128)] = lo
        wb[sub * nr:(sub + 1) * nr, pl.ds(c0 + 384, 128)] = hi

    def a_out(i, c):
        r0 = pl.multiple_of(i * TB, TB)
        lhs = ot[:, pl.ds(r0, TB)].T
        pieces = [(i * HP_IT + k, t, sub) for k in range(HP_IT) for t in range(3)
                  for sub in range(SUB)]
        slots = [(cc, rr) for rr in range(RS) for cc in range(CS)]
        spare = spare_idx[0]
        rb, cw = TB // RS, D // CS
        for si, (cc, rr) in enumerate(slots):
            a = jnp.dot(lhs[rr * rb:(rr + 1) * rb], pltpu.bitcast(awo[:, cc * cw:(cc + 1) * cw], BF),
                        preferred_element_type=F32)
            rows = pl.ds(pl.multiple_of(r0 + rr * rb, rb), rb)
            abuf[rows, cc * cw:(cc + 1) * cw] = a * gbuf[rows, :]
            stage[spare, 0:8, :] = pltpu.bitcast(a[0:8, 0:128], U32)
            for q, p in enumerate(pieces):
                if q * len(slots) // len(pieces) == si:
                    relayout(*p)
        return c

    with jax.named_scope("ph_aout"):
        jax.lax.fori_loop(0, nblk, a_out, 0)

    wob_cp.wait()

    NE, NO = 32, 48
    ri = jax.lax.broadcasted_iota(jnp.int32, (NE, L), 0)
    ci = jax.lax.broadcasted_iota(jnp.int32, (NE, L), 1)
    mask_e = (ri < M) | (ri >= ci)
    fill_e = NEG_B
    ri = jax.lax.broadcasted_iota(jnp.int32, (NO, 2 * L), 0)
    ci = jax.lax.broadcasted_iota(jnp.int32, (NO, 2 * L), 1)
    own = ((ri < L) & (ci >= L)) | ((ri >= L) & (ci < L))
    qi = jnp.where(ri < L, ri, ri - 8)
    ki = jnp.where(ci < L, ci, ci - L)
    mask_o = own & ((qi < M) | (qi >= ki))
    fill_o = jnp.where(own, NEG_B, -3e38)

    def qkv_dot(lhs, g):
        w = pltpu.bitcast(wb[:, g * GB * 384:(g + 1) * GB * 384], BF)
        return jnp.dot(lhs, w, preferred_element_type=F32)

    def qk_dots(qrows, kvrows):
        res = []
        for hh in range(GB):
            b = hh * 384
            q = (qrows[:, b:b + 128] * CB).astype(BF)
            k = kvrows[:, b + 128:b + 256].astype(BF)
            v = kvrows[:, b + 256:b + 384].astype(BF)
            s = jax.lax.dot_general(q, k, (((1,), (1,)), ((), ())), preferred_element_type=F32)
            res.append((s, v))
        return res

    def pv_dots(sv, mask, fill):
        outs = []
        for s, v in sv:
            s = jnp.where(mask, s, fill)
            mx = jnp.max(s, axis=1, keepdims=True)
            p = jnp.exp2(s - mx)
            l = jnp.sum(p, axis=1, keepdims=True)
            o = jnp.dot(p.astype(BF), v, preferred_element_type=F32)
            outs.append(o / l)
        return jnp.concatenate(outs, axis=1)

    def wo_dot(lhs, g):
        w = pltpu.bitcast(wob[g * GB * 64:(g + 1) * GB * 64, :], BF)
        return jnp.dot(lhs.astype(BF), w, preferred_element_type=F32)

    def run_step(lhs, rows_fn, mask, fill):
        qkv, sv, o = {}, {}, {}
        out = None
        qkv[0] = qkv_dot(lhs, 0)
        for g in range(NGB + WO_LAG):
            if g + 1 < NGB:
                qkv[g + 1] = qkv_dot(lhs, g + 1)
            if g < NGB:
                sv[g] = qk_dots(*rows_fn(qkv[g], g))
            if 0 <= g - PV_LAG < NGB:
                o[g - PV_LAG] = pv_dots(sv[g - PV_LAG], mask, fill)
            if 0 <= g - WO_LAG < NGB:
                d = wo_dot(o[g - WO_LAG], g - WO_LAG)
                out = d if out is None else out + d
        return out, qkv

    def pair(j, mem):
        t0 = pl.multiple_of(j * 2 * SEG, 2 * SEG)
        t1 = pl.multiple_of(j * 2 * SEG + SEG, SEG)
        x_e = ax[pl.ds(t0, 48), :].astype(F32)[:40]
        x_o = ax[pl.ds(t1, SEG), :].astype(F32)[8:]
        lhs_e = jnp.concatenate([mem, x_e], axis=0).astype(BF)
        out_e, qkv_e = run_step(lhs_e, lambda q, g: (q[:NE], q[:L]), mask_e, fill_e)
        mem1 = out_e[:M].astype(BF).astype(F32)
        lhs_o = jnp.concatenate([mem1, x_o], axis=0).astype(BF)

        def rows_o(q, g):
            e = qkv_e[g]
            seg_o = [q[:8], e[40:48], q[8:32]]
            return (jnp.concatenate(seg_o + [e[32:40]], axis=0),
                    jnp.concatenate([e[:L]] + seg_o, axis=0))

        out_o, _ = run_step(lhs_o, rows_o, mask_o, fill_o)
        b = jnp.concatenate([out_e[8:32], out_o[40:48], out_o[8:40]], axis=0)
        rows = pl.ds(t0, 2 * SEG)
        omg = jnp.concatenate([1.0 - gbuf[rows, :]] * (D // 128), axis=1)
        outbuf[rows, :] = (abuf[rows, :] + omg * b).astype(BF)
        pltpu.make_async_copy(outbuf.at[rows, :], out_hbm.at[rows, :], sem_out).start()
        return out_o[:M].astype(BF).astype(F32)

    with jax.named_scope("ph_pair"):
        jax.lax.fori_loop(0, N_PAIRS, pair, mem_ref[...].astype(F32))

    pltpu.make_async_copy(outbuf, out_hbm, sem_out).wait()


@functools.partial(jax.jit, static_argnames=("B_seg_len",))
def pallas_gated_mix__softmax_full_mha__memory_aug_recurrent_mem_tr__prompt_kernel(
    A_x: jax.Array,
    A_wqkv: jax.Array,
    A_wo: jax.Array,
    B_x: jax.Array,
    B_mem0: jax.Array,
    B_Wq: jax.Array,
    B_Wk: jax.Array,
    B_Wv: jax.Array,
    B_Wo: jax.Array,
    B_seg_len: int,
    gate_w: jax.Array,
):
    assert B_seg_len == SEG
    assert A_x.shape == (1, S, D)
    assert B_Wq.shape == (D, HB, DHB) and B_Wo.shape == (HB, DHB, D)

    any_spec = pl.BlockSpec(memory_space=pl.ANY)
    vmem_spec = pl.BlockSpec(memory_space=pltpu.VMEM)
    out = pl.pallas_call(
        _kernel,
        out_shape=jax.ShapeDtypeStruct((S, D), BF),
        in_specs=[any_spec, any_spec, any_spec, vmem_spec, any_spec, any_spec,
                  any_spec, any_spec, vmem_spec],
        out_specs=any_spec,
        scratch_shapes=[
            pltpu.VMEM((S, D), BF),
            pltpu.VMEM((3, D // 2, D), U32),
            pltpu.VMEM((D // 2, D), U32),
            pltpu.VMEM((S // 2, D), U32),
            pltpu.VMEM((D, S), BF),
            pltpu.VMEM((D // 2, S), U32),
            pltpu.VMEM((D, S), BF),
            pltpu.VMEM((S, D), F32),
            pltpu.VMEM((S, 128), F32),
            pltpu.VMEM((D // 2, HB * 384), U32),
            pltpu.VMEM((HB * DHB // 2, D), U32),
            pltpu.VMEM((N_HP * 6 + 1, D // 2, 128), U32),
            pltpu.VMEM((S, D), BF),
            pltpu.VMEM((AHEAD, KB, QB), F32),
            pltpu.SMEM((1,), jnp.int32),
            pltpu.SemaphoreType.DMA((S // TB + 9,)),
            pltpu.SemaphoreType.DMA((N_HP,)),
            pltpu.SemaphoreType.DMA(()),
        ],
        compiler_params=pltpu.CompilerParams(vmem_limit_bytes=124 * 1024 * 1024),
    )(A_x.reshape(S, D), A_wqkv, A_wo, B_mem0.reshape(M, D),
      *[w.reshape(D // 2, 2, HB, DHB) for w in (B_Wq, B_Wk, B_Wv)],
      B_Wo.reshape(HB * DHB, D), gate_w)
    return out.reshape(1, S, D)
```

```python
import functools
import math

import jax
import jax.numpy as jnp
import jax.experimental.pallas as pl
import jax.experimental.pallas.tpu as pltpu

BF = jnp.bfloat16
F32 = jnp.float32
U32 = jnp.uint32

S = 2048
D = 1024
HA, DHA = 32, 32
HB, DHB = 32, 128
M = 8
SEG = 32
L = M + SEG

LOG2E = math.log2(math.e)
CA = DHA ** -0.5 * LOG2E
CB = DHB ** -0.5 * LOG2E
NEG_B = -1e9 * LOG2E

TB = 512
QB = 256
KB = 128
AHEAD = 4
UN = 16
GB = 2
NGB = HB // GB
PV_LAG, WO_LAG = 2, 3
NQ = S // QB
NK = S // KB
N_UNITS = HA * NQ
N_PAIRS = S // (2 * SEG)
N_HP = HB // 2


def _tree(op, xs):
    xs = list(xs)
    while len(xs) > 1:
        nxt = [op(xs[i], xs[i + 1]) for i in range(0, len(xs) - 1, 2)]
        if len(xs) % 2:
            nxt.append(xs[-1])
        xs = nxt
    return xs[0]


def _kernel(ax_hbm, wqkv_hbm, awo_hbm, mem_ref, bwq_hbm, bwk_hbm, bwv_hbm,
            bwo_hbm, gw_ref, out_hbm,
            ax, wqkv, awo, kbuf, qt, vt, ot, abuf, gbuf, wb, wob, stage, outbuf, scarry, spare_idx,
            sem_in, sem_st, sem_out):
    nblk = S // TB

    def ax_cp(i):
        r0 = pl.multiple_of(i * TB, TB)
        return pltpu.make_async_copy(ax_hbm.at[pl.ds(r0, TB), :], ax.at[pl.ds(r0, TB), :],
                                     sem_in.at[i])

    wqkv_u32 = wqkv_hbm.bitcast(U32)
    NC = 4
    CW = D // NC

    def wk_cp(c):
        c0 = pl.multiple_of(c * CW, CW)
        return pltpu.make_async_copy(wqkv_u32.at[:, pl.ds(D + c0, CW)],
                                     wqkv.at[1, :, pl.ds(c0, CW)], sem_in.at[nblk + 5 + c])

    def wqkv_cp(t):
        return pltpu.make_async_copy(wqkv_u32.at[:, pl.ds(t * D, D)], wqkv.at[t],
                                     sem_in.at[nblk + t])

    awo_cp = pltpu.make_async_copy(awo_hbm.bitcast(U32), awo, sem_in.at[nblk + 3])
    wob_cp = pltpu.make_async_copy(bwo_hbm.bitcast(U32), wob, sem_in.at[nblk + 4])

    bw_u32 = [r.bitcast(U32) for r in (bwq_hbm, bwk_hbm, bwv_hbm)]

    def stage_cp(hp, t, par):
        return pltpu.make_async_copy(bw_u32[t].at[:, par, hp, :],
                                     stage.at[(hp * 3 + t) * 2 + par], sem_st.at[hp])

    HB0 = TB // 2

    def ax0_cp(half):
        return pltpu.make_async_copy(ax_hbm.at[pl.ds(half * HB0, HB0), :],
                                     ax.at[pl.ds(half * HB0, HB0), :], sem_in.at[half * (nblk + 1)])

    spare_idx[0] = N_HP * 6
    ax0_cp(0).start()
    for c in range(NC):
        wk_cp(c).start()
    ax0_cp(1).start()
    for i in range(1, nblk):
        ax_cp(i).start()
    wqkv_cp(0).start()
    wqkv_cp(2).start()

    ax0_cp(0).wait()

    def k_proj0(c, carry):
        wk_cp(c).wait()
        c0 = pl.multiple_of(c * CW, CW)
        k = jnp.dot(ax[0:HB0, :], pltpu.bitcast(wqkv[1, :, pl.ds(c0, CW)], BF),
                    preferred_element_type=F32)
        kbuf[0:HB0 // 2, pl.ds(c0, CW)] = pltpu.bitcast(k.astype(BF), U32)
        return carry

    def k_proj(i, c):
        ax_cp(i).wait()
        r0 = pl.multiple_of(i * TB, TB)
        rh = pl.multiple_of(i * (TB // 2), TB // 2)
        k = jnp.dot(ax[pl.ds(r0, TB), :], pltpu.bitcast(wqkv[1], BF), preferred_element_type=F32)
        kbuf[pl.ds(rh, TB // 2), :] = pltpu.bitcast(k.astype(BF), U32)
        return c

    with jax.named_scope("ph_kproj0"):
        jax.lax.fori_loop(0, NC, k_proj0, 0)
        ax0_cp(1).wait()
        k = jnp.dot(ax[HB0:TB, :], pltpu.bitcast(wqkv[1], BF), preferred_element_type=F32)
        kbuf[HB0 // 2:TB // 2, :] = pltpu.bitcast(k.astype(BF), U32)
    with jax.named_scope("ph_kproj"):
        jax.lax.fori_loop(1, nblk, k_proj, 0)

    wqkv_cp(0).wait()
    wqkv_cp(2).wait()
    def start_stage(hp_lo, hp_hi):
        for hp in range(hp_lo, hp_hi):
            for t in range(3):
                for par in range(2):
                    stage_cp(hp, t, par).start(priority=1)

    start_stage(0, N_HP // 4)
    awo_cp.start(priority=1)
    wob_cp.start(priority=1)

    def qv_proj(i, c):
        r0 = pl.multiple_of(i * TB, TB)
        xb = ax[pl.ds(r0, TB), :]
        q = jnp.dot(xb, pltpu.bitcast(wqkv[0], BF), preferred_element_type=F32) * CA
        qt[:, pl.ds(r0, TB)] = q.T.astype(BF)
        v = jnp.dot(xb, pltpu.bitcast(wqkv[2], BF), preferred_element_type=F32)
        vt[:, pl.ds(r0, TB)] = pltpu.bitcast(v.T.astype(BF), U32)
        z = jnp.sum(xb.astype(F32) * gw_ref[...].astype(F32).reshape(1, D), axis=1, keepdims=True)
        gbuf[pl.ds(r0, TB), :] = jnp.broadcast_to(1.0 / (1.0 + jnp.exp(-z)), (TB, 128))
        return c

    with jax.named_scope("ph_qvproj"):
        jax.lax.fori_loop(0, nblk, qv_proj, 0)

    start_stage(N_HP // 4, 3 * N_HP // 4)

    def unit_setup(u):
        h = u % HA
        g0 = pl.multiple_of((h // 4) * 128, 128)
        h0 = pl.multiple_of(h * DHA, DHA)
        q0 = pl.multiple_of((u // HA) * QB, QB)
        qg = pltpu.bitcast(qt[pl.ds(g0, 128), pl.ds(q0, QB)], U32)
        rows = jax.lax.broadcasted_iota(jnp.int32, (64, QB), 0)
        qm = pltpu.bitcast(jnp.where(rows // 16 == h % 4, qg, U32(0)), BF)
        return qm, g0, h0, q0

    def qk_chunk(setup, j):
        qm, g0, _, _ = setup
        kb = pltpu.bitcast(kbuf[j * KB // 2:(j + 1) * KB // 2, pl.ds(g0, 128)], BF)
        return jnp.dot(kb, qm, preferred_element_type=F32)

    def attn_iter(it, c):
        @pl.when(it == 4)
        def _():
            start_stage(3 * N_HP // 4, N_HP)

        setup = [unit_setup(it * UN + k) for k in range(UN)]
        setup_next = unit_setup(jnp.minimum(it * UN + UN, N_UNITS - 1))
        items = [(uu, j) for uu in range(UN) for j in range(NK)]
        n = len(items)
        state = {}

        def pv(i, p, al, l):
            uu, j = items[i]
            _, _, h0, q0 = setup[uu]
            hh0 = pl.multiple_of(h0 // 2, DHA // 2)
            vtb = pltpu.bitcast(vt[pl.ds(hh0, DHA // 2), j * KB:(j + 1) * KB], BF)
            d = jnp.dot(vtb, p, preferred_element_type=F32)
            acc = d if j == 0 else state["acc"] * al + d
            state["acc"] = acc
            if j == NK - 1:
                o = acc / jnp.sum(l, axis=0, keepdims=True)
                ot[pl.ds(h0, DHA), pl.ds(q0, QB)] = o.astype(BF)

        ss = {i: scarry[i] for i in range(AHEAD)}
        m = l = None
        pend = None
        for i, (uu, j) in enumerate(items):
            if i + AHEAD < n:
                uu2, j2 = items[i + AHEAD]
                ss[i + AHEAD] = qk_chunk(setup[uu2], j2)
            else:
                scarry[i + AHEAD - n] = qk_chunk(setup_next, i + AHEAD - n)
            if pend is not None:
                pv(*pend)
            s = ss.pop(i)
            bm = _tree(jnp.maximum, [s[8 * r:8 * r + 8] for r in range(KB // 8)])
            bm = jnp.max(bm, axis=0, keepdims=True)
            if j == 0:
                m, al = bm, None
                p = jnp.exp2(s - m)
                l = _tree(jnp.add, [p[8 * r:8 * r + 8] for r in range(KB // 8)])
            else:
                mn = jnp.maximum(m, bm)
                al = jnp.exp2(m - mn)
                p = jnp.exp2(s - mn)
                l = l * al + _tree(jnp.add, [p[8 * r:8 * r + 8] for r in range(KB // 8)])
                m = mn
            pend = (i, p.astype(BF), al, l)
        pv(*pend)
        return c

    setup0 = unit_setup(0)
    for j in range(AHEAD):
        scarry[j] = qk_chunk(setup0, j)
    with jax.named_scope("ph_attn"):
        jax.lax.fori_loop(0, N_UNITS // UN, attn_iter, 0)

    awo_cp.wait()
    for hp in range(N_HP):
        pltpu.make_async_copy(stage.at[pl.ds(hp * 6, 6)], stage.at[pl.ds(hp * 6, 6)],
                              sem_st.at[hp]).wait()

    RS, CS, SUB = 4, 8, 32
    HP_IT = N_HP // nblk

    def relayout(hp, t, sub):
        nr = D // 2 // SUB
        ev = stage[(hp * 3 + t) * 2, sub * nr:(sub + 1) * nr, :]
        od = stage[(hp * 3 + t) * 2 + 1, sub * nr:(sub + 1) * nr, :]
        lo = (ev & U32(0xFFFF)) | (od << 16)
        hi = (ev >> 16) | (od & U32(0xFFFF0000))
        c0 = pl.multiple_of(hp * 768 + t * 128, 128)
        wb[sub * nr:(sub + 1) * nr, pl.ds(c0, 128)] = lo
        wb[sub * nr:(sub + 1) * nr, pl.ds(c0 + 384, 128)] = hi

    def a_out(i, c):
        r0 = pl.multiple_of(i * TB, TB)
        lhs = ot[:, pl.ds(r0, TB)].T
        pieces = [(i * HP_IT + k, t, sub) for k in range(HP_IT) for t in range(3)
                  for sub in range(SUB)]
        slots = [(cc, rr) for rr in range(RS) for cc in range(CS)]
        spare = spare_idx[0]
        rb, cw = TB // RS, D // CS
        for si, (cc, rr) in enumerate(slots):
            a = jnp.dot(lhs[rr * rb:(rr + 1) * rb], pltpu.bitcast(awo[:, cc * cw:(cc + 1) * cw], BF),
                        preferred_element_type=F32)
            rows = pl.ds(pl.multiple_of(r0 + rr * rb, rb), rb)
            abuf[rows, cc * cw:(cc + 1) * cw] = a * gbuf[rows, :]
            stage[spare, 0:8, :] = pltpu.bitcast(a[0:8, 0:128], U32)
            for q, p in enumerate(pieces):
                if q * len(slots) // len(pieces) == si:
                    relayout(*p)
        return c

    with jax.named_scope("ph_aout"):
        jax.lax.fori_loop(0, nblk, a_out, 0)

    wob_cp.wait()

    NE, NO = 32, 48
    ri = jax.lax.broadcasted_iota(jnp.int32, (NE, L), 0)
    ci = jax.lax.broadcasted_iota(jnp.int32, (NE, L), 1)
    mask_e = (ri < M) | (ri >= ci)
    fill_e = NEG_B
    ri = jax.lax.broadcasted_iota(jnp.int32, (NO, 2 * L), 0)
    ci = jax.lax.broadcasted_iota(jnp.int32, (NO, 2 * L), 1)
    own = ((ri < L) & (ci >= L)) | ((ri >= L) & (ci < L))
    qi = jnp.where(ri < L, ri, ri - 8)
    ki = jnp.where(ci < L, ci, ci - L)
    mask_o = own & ((qi < M) | (qi >= ki))
    fill_o = jnp.where(own, NEG_B, -3e38)

    def qkv_dot(lhs, g):
        w = pltpu.bitcast(wb[:, g * GB * 384:(g + 1) * GB * 384], BF)
        return jnp.dot(lhs, w, preferred_element_type=F32)

    def qk_dots(qrows, kvrows):
        res = []
        for hh in range(GB):
            b = hh * 384
            q = (qrows[:, b:b + 128] * CB).astype(BF)
            k = kvrows[:, b + 128:b + 256].astype(BF)
            v = kvrows[:, b + 256:b + 384].astype(BF)
            s = jax.lax.dot_general(q, k, (((1,), (1,)), ((), ())), preferred_element_type=F32)
            res.append((s, v))
        return res

    def pv_dots(sv, mask, fill):
        outs = []
        for s, v in sv:
            s = jnp.where(mask, s, fill)
            mx = jnp.max(s, axis=1, keepdims=True)
            p = jnp.exp2(s - mx)
            l = jnp.sum(p, axis=1, keepdims=True)
            o = jnp.dot(p.astype(BF), v, preferred_element_type=F32)
            outs.append(o / l)
        return jnp.concatenate(outs, axis=1)

    def wo_dot(lhs, g):
        w = pltpu.bitcast(wob[g * GB * 64:(g + 1) * GB * 64, :], BF)
        return jnp.dot(lhs.astype(BF), w, preferred_element_type=F32)

    def run_step(lhs, rows_fn, mask, fill):
        qkv, sv, o = {}, {}, {}
        out = None
        qkv[0] = qkv_dot(lhs, 0)
        for g in range(NGB + WO_LAG):
            if g + 1 < NGB:
                qkv[g + 1] = qkv_dot(lhs, g + 1)
            if g < NGB:
                sv[g] = qk_dots(*rows_fn(qkv[g], g))
            if 0 <= g - PV_LAG < NGB:
                o[g - PV_LAG] = pv_dots(sv[g - PV_LAG], mask, fill)
            if 0 <= g - WO_LAG < NGB:
                d = wo_dot(o[g - WO_LAG], g - WO_LAG)
                out = d if out is None else out + d
        return out, qkv

    def pair(j, mem):
        t0 = pl.multiple_of(j * 2 * SEG, 2 * SEG)
        t1 = pl.multiple_of(j * 2 * SEG + SEG, SEG)
        x_e = ax[pl.ds(t0, 48), :].astype(F32)[:40]
        x_o = ax[pl.ds(t1, SEG), :].astype(F32)[8:]
        lhs_e = jnp.concatenate([mem, x_e], axis=0).astype(BF)
        out_e, qkv_e = run_step(lhs_e, lambda q, g: (q[:NE], q[:L]), mask_e, fill_e)
        mem1 = out_e[:M].astype(BF).astype(F32)
        lhs_o = jnp.concatenate([mem1, x_o], axis=0).astype(BF)

        def rows_o(q, g):
            e = qkv_e[g]
            seg_o = [q[:8], e[40:48], q[8:32]]
            return (jnp.concatenate(seg_o + [e[32:40]], axis=0),
                    jnp.concatenate([e[:L]] + seg_o, axis=0))

        out_o, _ = run_step(lhs_o, rows_o, mask_o, fill_o)
        b = jnp.concatenate([out_e[8:32], out_o[40:48], out_o[8:40]], axis=0)
        rows = pl.ds(t0, 2 * SEG)
        omg = jnp.concatenate([1.0 - gbuf[rows, :]] * (D // 128), axis=1)
        outbuf[rows, :] = (abuf[rows, :] + omg * b).astype(BF)
        pltpu.make_async_copy(outbuf.at[rows, :], out_hbm.at[rows, :], sem_out).start()
        return out_o[:M].astype(BF).astype(F32)

    with jax.named_scope("ph_pair"):
        jax.lax.fori_loop(0, N_PAIRS, pair, mem_ref[...].astype(F32))

    pltpu.make_async_copy(outbuf, out_hbm, sem_out).wait()


@functools.partial(jax.jit, static_argnames=("B_seg_len",))
def pallas_gated_mix__softmax_full_mha__memory_aug_recurrent_mem_tr__prompt_kernel(
    A_x: jax.Array,
    A_wqkv: jax.Array,
    A_wo: jax.Array,
    B_x: jax.Array,
    B_mem0: jax.Array,
    B_Wq: jax.Array,
    B_Wk: jax.Array,
    B_Wv: jax.Array,
    B_Wo: jax.Array,
    B_seg_len: int,
    gate_w: jax.Array,
):
    assert B_seg_len == SEG
    assert A_x.shape == (1, S, D)
    assert B_Wq.shape == (D, HB, DHB) and B_Wo.shape == (HB, DHB, D)

    any_spec = pl.BlockSpec(memory_space=pl.ANY)
    vmem_spec = pl.BlockSpec(memory_space=pltpu.VMEM)
    out = pl.pallas_call(
        _kernel,
        out_shape=jax.ShapeDtypeStruct((S, D), BF),
        in_specs=[any_spec, any_spec, any_spec, vmem_spec, any_spec, any_spec,
                  any_spec, any_spec, vmem_spec],
        out_specs=any_spec,
        scratch_shapes=[
            pltpu.VMEM((S, D), BF),
            pltpu.VMEM((3, D // 2, D), U32),
            pltpu.VMEM((D // 2, D), U32),
            pltpu.VMEM((S // 2, D), U32),
            pltpu.VMEM((D, S), BF),
            pltpu.VMEM((D // 2, S), U32),
            pltpu.VMEM((D, S), BF),
            pltpu.VMEM((S, D), F32),
            pltpu.VMEM((S, 128), F32),
            pltpu.VMEM((D // 2, HB * 384), U32),
            pltpu.VMEM((HB * DHB // 2, D), U32),
            pltpu.VMEM((N_HP * 6 + 1, D // 2, 128), U32),
            pltpu.VMEM((S, D), BF),
            pltpu.VMEM((AHEAD, KB, QB), F32),
            pltpu.SMEM((1,), jnp.int32),
            pltpu.SemaphoreType.DMA((S // TB + 9,)),
            pltpu.SemaphoreType.DMA((N_HP,)),
            pltpu.SemaphoreType.DMA(()),
        ],
        compiler_params=pltpu.CompilerParams(vmem_limit_bytes=124 * 1024 * 1024),
    )(A_x.reshape(S, D), A_wqkv, A_wo, B_mem0.reshape(M, D),
      *[w.reshape(D // 2, 2, HB, DHB) for w in (B_Wq, B_Wk, B_Wv)],
      B_Wo.reshape(HB * DHB, D), gate_w)
    return out.reshape(1, S, D)
```
